```python
import jax
import jax.numpy as jnp

def _softmax(x, axis=-1):
    return jax.nn.softmax(x, axis=axis)

def _gelu(x):
    return jax.nn.gelu(x, approximate=True)

def _silu(x):
    return jax.nn.silu(x)

def _sigmoid(x):
    return jax.nn.sigmoid(x)

def _layernorm(x, axis=-1, eps=1e-05):
    m = jnp.mean(x, axis=axis, keepdims=True)
    v = jnp.var(x, axis=axis, keepdims=True)
    return (x - m) / jnp.sqrt(v + eps)

def _scatter_add(tgt, idx, src, axis=0):
    return tgt.at[idx].add(src)

def _segment_sum(src, seg, n):
    return jax.ops.segment_sum(src, seg, n)

class _Rng:

    def __init__(self, key):
        self._k = key

    def _next(self):
        self._k, sub = jax.random.split(self._k)
        return sub

    def normal(self, shape):
        return jax.random.normal(self._next(), shape, dtype=jnp.bfloat16)

    def randint(self, lo, hi, shape):
        return jax.random.randint(self._next(), shape, lo, hi, dtype=jnp.int32)

    def uniform(self, shape, lo=0.0, hi=1.0):
        return jax.random.uniform(self._next(), shape, jnp.bfloat16, lo, hi)

    def permutation(self, n):
        return jax.random.permutation(self._next(), n)
kernel_name = 'sequential_preLN__memory_aug_recurrent_mem_tr__moe_arch_mod__prompt'

def setup_inputs():
    _rng = _Rng(jax.random.key(int.from_bytes(__import__("os").urandom(4), "little")))
    _w = lambda a: (lambda t: t.astype(jnp.bfloat16) if jnp.issubdtype(t.dtype, jnp.floating) else t)(jnp.asarray(a))

    def _A_setup():
        B, S, Dm = (1, 2048, 512)
        H, Dh = (32, 128)
        M, seg = (8, 32)
        seg = min(seg, S)
        S = S // seg * seg
        return {'x': _w((lambda *s: _rng.normal(s) * 0.05)(B, S, Dm)), 'mem0': _w((lambda *s: _rng.normal(s) * 0.05)(B, M, Dm)), 'Wq': _w((lambda *s: _rng.normal(s) * 0.05)(Dm, H, Dh) * Dm ** (-0.5)), 'Wk': _w((lambda *s: _rng.normal(s) * 0.05)(Dm, H, Dh) * Dm ** (-0.5)), 'Wv': _w((lambda *s: _rng.normal(s) * 0.05)(Dm, H, Dh) * Dm ** (-0.5)), 'Wo': _w((lambda *s: _rng.normal(s) * 0.05)(H, Dh, Dm) * (H * Dh) ** (-0.5)), 'seg_len': seg}
    _A_in = _A_setup()

    def _B_setup():
        B, S, D, F, C = (1, 2048, 512, 1792, 2)
        return {'x': _w((lambda *s: _rng.normal(s) * 0.05)(B, S, D)), 'w_r': _w((lambda *s: _rng.normal(s) * 0.05)(D)), 'w_gate': _w((lambda *s: _rng.normal(s) * 0.05)(D, F)), 'w_up': _w((lambda *s: _rng.normal(s) * 0.05)(D, F)), 'w_down': _w((lambda *s: _rng.normal(s) * 0.05)(F, D))}
    _B_in = _B_setup()
    return {'A_x': _A_in['x'], 'A_mem0': _A_in['mem0'], 'A_Wq': _A_in['Wq'], 'A_Wk': _A_in['Wk'], 'A_Wv': _A_in['Wv'], 'A_Wo': _A_in['Wo'], 'A_seg_len': _A_in['seg_len'], 'B_x': _B_in['x'], 'B_w_r': _B_in['w_r'], 'B_w_gate': _B_in['w_gate'], 'B_w_up': _B_in['w_up'], 'B_w_down': _B_in['w_down']}

def reference(A_x, A_mem0, A_Wq, A_Wk, A_Wv, A_Wo, A_seg_len, B_x, B_w_r, B_w_gate, B_w_up, B_w_down):

    def _A_ref(x, mem0, Wq, Wk, Wv, Wo, seg_len):
        B, S, Dm = x.shape
        H, Dh = (Wq.shape[1], Wq.shape[2])
        M = mem0.shape[1]
        scale = Dh ** (-0.5)
        n_seg = S // seg_len
        L = M + seg_len
        idx = jnp.arange(L)
        mask = (idx[:, None] < M) | (idx[:, None] >= idx[None, :])
        mem = mem0
        outs = []
        for s in range(n_seg):
            xs = x[:, s * seg_len:(s + 1) * seg_len, :].copy()
            h = jnp.concatenate([mem, xs], axis=1)
            q = jnp.einsum('btd,dhe->bhte', h, Wq)
            k = jnp.einsum('btd,dhe->bhte', h, Wk)
            v = jnp.einsum('btd,dhe->bhte', h, Wv)
            scores = jnp.einsum('bhqe,bhke->bhqk', q, k) * scale
            scores = jnp.where(mask[None, None], scores, -1000000000.0)
            p = _softmax(scores, axis=-1)
            o = jnp.einsum('bhqk,bhke->bhqe', p, v)
            o = jnp.einsum('bhte,hed->btd', o, Wo)
            mem = o[:, :M, :].copy()
            outs.append(o[:, M:, :])
        return jnp.concatenate(outs, axis=1)

    def _B_ref(x, w_r, w_gate, w_up, w_down):
        B, S, D = x.shape
        C = 2
        r = x @ w_r
        idx = jnp.argsort(-r, axis=-1)[:, :C]
        idx_e = jnp.repeat(idx.reshape(B, C, 1), D, axis=2)
        x_sel = jnp.take_along_axis(x, idx_e, axis=1)
        g = _silu(x_sel @ w_gate)
        u = x_sel @ w_up
        y = g * u @ w_down
        r_sel = _sigmoid(jnp.take_along_axis(r, idx, axis=1))
        y = y * r_sel.reshape(B, C, 1)
        b_off = (jnp.arange(B) * S).reshape(B, 1)
        flat_idx = (idx + b_off).reshape(B * C)
        zero = (x * 0.0).reshape(B * S, D)
        upd = _scatter_add(zero, flat_idx, y.reshape(B * C, D), axis=0)
        return x + upd.reshape(B, S, D)
    x = A_x
    h = x + _A_ref(_layernorm(x, axis=-1), A_mem0, A_Wq, A_Wk, A_Wv, A_Wo, A_seg_len)
    h2 = h + _B_ref(_layernorm(h, axis=-1), B_w_r, B_w_gate, B_w_up, B_w_down)
    return h2
```

```python
import functools

import jax
import jax.numpy as jnp
import numpy as np
from jax import lax
import jax.experimental.pallas as pl
import jax.experimental.pallas.tpu as pltpu

F32 = jnp.float32
BF16 = jnp.bfloat16
U32 = jnp.uint32

_NN = (((1,), (0,)), ((), ()))
_NT = (((1,), (1,)), ((), ()))


def _rb(x):
    return x.astype(BF16).astype(F32)


def _layernorm(x):
    n = x.shape[-1]
    m = jnp.sum(x, axis=-1, keepdims=True) * (1.0 / n)
    xc = x - m
    v = jnp.sum(xc * xc, axis=-1, keepdims=True) * (1.0 / n)
    sd = _rb(jnp.sqrt(_rb(_rb(v) + 1e-5)))
    return _rb(_rb(x - _rb(m)) / sd)


def _mm(a, w_u32):
    return lax.dot_general(a, pltpu.bitcast(w_u32, BF16), _NN, preferred_element_type=F32)


def _kernel(x_hbm, mem_ref, wq_hbm, wk_hbm, wv_hbm, wo_hbm, wr_ref, wg_hbm, wu_hbm, wd_hbm,
            out_hbm,
            xb, xn, hs, raw, wqkv, wo_raw, wo, wg, wu, wd, ob, sems,
            *, seg, n_mem, n_heads, dh):
    S, D = xb.shape
    n_seg = S // seg
    L = seg + n_mem
    G = 4
    NG = n_heads // G
    scale = float(dh) ** -0.5

    cx = pltpu.make_async_copy(x_hbm, xb, sems.at[0])
    cx.start()
    cw = []
    for m, w in enumerate((wk_hbm, wq_hbm, wv_hbm)):
        for half in range(2):
            c = pltpu.make_async_copy(w.at[:, pl.ds(16 * half, 16), :], raw.at[2 * m + half], sems.at[1 + 2 * m + half])
            c.start()
            cw.append(c)
    co = pltpu.make_async_copy(wo_hbm, wo_raw, sems.at[7])
    co.start()
    cf = [pltpu.make_async_copy(a, b, sems.at[8 + i]) for i, (a, b) in enumerate(((wg_hbm, wg), (wu_hbm, wu), (wd_hbm, wd)))]
    for c in cf:
        c.start()

    cx.wait()

    def ln_body(i, _):
        r = pl.ds(pl.multiple_of(i * 64, 64), 64)
        xn[r, :] = _layernorm(xb[r, :].astype(F32))
    lax.fori_loop(0, S // 64, ln_body, None)

    for c in range(6):
        cw[c].wait()

        def rl_body(i, _, c=c):
            a = pltpu.bitcast(raw[c, pl.ds(i * 16, 16)], U32)
            t = jnp.swapaxes(a, 0, 1)
            rows = pl.ds(pl.multiple_of(i * 8, 8), 8)
            for j in range(8):
                lo = pltpu.bitcast(t[j] << 16, F32).astype(BF16)
                hi = pltpu.bitcast(t[j] & np.uint32(0xFFFF0000), F32).astype(BF16)
                g = (c // 2) * NG + (c % 2) * 4 + j // 2
                col = (j % 2) * 256
                wqkv[g, rows, col:col + 128] = pltpu.bitcast(lo, U32)
                wqkv[g, rows, col + 128:col + 256] = pltpu.bitcast(hi, U32)
        lax.fori_loop(0, D // 16, rl_body, None)

    co.wait()

    def wo_body(g, _):
        wo[g] = pltpu.bitcast(wo_raw[pl.ds(pl.multiple_of(g * 512, 512), 512), :], U32)
    lax.fori_loop(0, NG, wo_body, None)

    row = lax.broadcasted_iota(jnp.int32, (L, L), 0)
    col = lax.broadcasted_iota(jnp.int32, (L, L), 1)
    mask = (row >= seg) | (col >= seg) | (row >= col)
    c_exp = scale * float(np.log2(np.e))
    neg = -1e9 / scale

    def step(s, mem):
        r = pl.ds(pl.multiple_of(s * seg, seg), seg)
        h = jnp.concatenate([xn[r, :], mem], axis=0)
        k, q, v, p, l, o = {}, {}, {}, {}, {}, {}
        acc = [None]

        def K(g):
            k[g] = _mm(h, wqkv[g])

        def Q(g):
            q[g] = _mm(h, wqkv[NG + g])

        def V(g):
            v[g] = _mm(h, wqkv[2 * NG + g])

        def Sc(g):
            for i in range(G):
                cs = slice(i * dh, (i + 1) * dh)
                sc = lax.dot_general(q[g][:, cs], k[g][:, cs].astype(BF16), _NT, preferred_element_type=F32)
                sc = jnp.where(mask, sc, neg)
                e = jnp.exp2((sc - jnp.max(sc, axis=-1, keepdims=True)) * c_exp)
                p[g, i] = e
                l[g, i] = jnp.sum(e, axis=-1, keepdims=True)

        def PV(g):
            os_ = []
            for i in range(G):
                cs = slice(i * dh, (i + 1) * dh)
                t = lax.dot_general(p[g, i], v[g][:, cs].astype(BF16), _NN, preferred_element_type=F32)
                os_.append(t * pl.reciprocal(l[g, i], approx=False))
            o[g] = jnp.concatenate(os_, axis=1)

        def O(g):
            t = _mm(o[g], wo[g])
            acc[0] = t if acc[0] is None else acc[0] + t

        K(0); Q(0); V(0)
        for g in range(1, NG):
            K(g); Sc(g - 1); Q(g); V(g); PV(g - 1)
        O(0); Sc(NG - 1); O(1); O(2); PV(NG - 1)
        for g in range(3, NG):
            O(g)
        hs[r, :] = acc[0][:seg]
        return _rb(acc[0][seg:])

    lax.fori_loop(0, n_seg, step, mem_ref[...].astype(F32))

    wr = wr_ref[...].astype(F32)
    wr = jnp.concatenate([wr[i:i + 1, :] for i in range(D // 128)], axis=1)
    sub = lax.broadcasted_iota(jnp.int32, (8, 128), 0)

    def post(i, carry):
        b1, i1, b2, i2 = carry
        r = pl.ds(pl.multiple_of(i * 64, 64), 64)
        h = _rb(xb[r, :].astype(F32) + _rb(hs[r, :]))
        hs[r, :] = h
        hn = _layernorm(h)
        ob[r, :] = (h + hn).astype(BF16)
        rr = _rb(jnp.sum(hn * wr, axis=-1, keepdims=True))
        for j in range(8):
            val = jnp.broadcast_to(rr[8 * j:8 * j + 8], (8, 128))
            idx = sub + (i * 64 + 8 * j)
            g1 = val > b1
            g2 = val > b2
            b2 = jnp.where(g1, b1, jnp.where(g2, val, b2))
            i2 = jnp.where(g1, i1, jnp.where(g2, idx, i2))
            b1 = jnp.where(g1, val, b1)
            i1 = jnp.where(g1, idx, i1)
        return b1, i1, b2, i2

    ninf = jnp.full((8, 128), -jnp.inf, F32)
    b1, i1, b2, i2 = lax.fori_loop(0, S // 64, post, (ninf, sub, ninf, sub + 8))
    big = np.int32(1 << 30)
    m1 = jnp.max(b1, axis=0, keepdims=True)
    t1 = jnp.min(jnp.where(b1 == m1, i1, big), axis=0, keepdims=True)
    won = i1 == t1
    cb = jnp.where(won, b2, b1)
    ci = jnp.where(won, i2, i1)
    m2 = jnp.max(cb, axis=0, keepdims=True)
    t2 = jnp.min(jnp.where(cb == m2, ci, big), axis=0, keepdims=True)
    idx1 = jnp.clip(t1[0, 0], 0, S - 1)
    idx2 = jnp.clip(t2[0, 0], 0, S - 1)

    for c in cf:
        c.wait()
    base1 = pl.multiple_of((idx1 // 16) * 16, 16)
    base2 = pl.multiple_of((idx2 // 16) * 16, 16)
    h = jnp.concatenate([hs[pl.ds(base1, 16), :], hs[pl.ds(base2, 16), :]], axis=0)
    hn = _layernorm(h)
    hb = hn.astype(BF16)
    gt = _rb(jnp.dot(hb, wg[...], preferred_element_type=F32))
    up = _rb(jnp.dot(hb, wu[...], preferred_element_type=F32))
    a = _rb(gt * _rb(jax.nn.sigmoid(gt))) * up
    y = _rb(jnp.dot(a.astype(BF16), wd[...], preferred_element_type=F32))
    rr = _rb(jnp.sum(hn * wr, axis=-1, keepdims=True))
    y = _rb(y * _rb(jax.nn.sigmoid(rr)))
    ri = lax.broadcasted_iota(jnp.int32, (32, D), 0)
    gi = jnp.where(ri < 16, ri + base1, ri + (base2 - 16))
    sel = (gi == idx1) | (gi == idx2)
    res = (h + _rb(hn + jnp.where(sel, y, 0.0))).astype(BF16)
    ob[pl.ds(base1, 16), :] = res[:16]
    ob[pl.ds(base2, 16), :] = res[16:]
    cout = pltpu.make_async_copy(ob, out_hbm, sems.at[11])
    cout.start()
    cout.wait()


@functools.partial(jax.jit, static_argnames=("A_seg_len",))
def pallas_sequential_preLN__memory_aug_recurrent_mem_tr__moe_arch_mod__prompt_kernel(
    A_x, A_mem0, A_Wq, A_Wk, A_Wv, A_Wo, A_seg_len, B_x, B_w_r, B_w_gate, B_w_up, B_w_down,
):
    del B_x
    _, S, D = A_x.shape
    _, H, Dh = A_Wq.shape
    M = A_mem0.shape[1]
    F = B_w_gate.shape[1]
    any_spec = pl.BlockSpec(memory_space=pl.ANY)
    vmem_spec = pl.BlockSpec(memory_space=pltpu.VMEM)
    out = pl.pallas_call(
        functools.partial(_kernel, seg=int(A_seg_len), n_mem=M, n_heads=H, dh=Dh),
        out_shape=jax.ShapeDtypeStruct((S, D), A_x.dtype),
        in_specs=[any_spec, vmem_spec, any_spec, any_spec, any_spec, any_spec, vmem_spec, any_spec, any_spec, any_spec],
        out_specs=any_spec,
        scratch_shapes=[
            pltpu.VMEM((S, D), BF16),
            pltpu.VMEM((S, D), F32),
            pltpu.VMEM((S, D), F32),
            pltpu.VMEM((6, D, 16, Dh), BF16),
            pltpu.VMEM((3 * H // 4, D // 2, 4 * Dh), U32),
            pltpu.VMEM((H * Dh, D), BF16),
            pltpu.VMEM((H // 4, 2 * Dh, D), U32),
            pltpu.VMEM((D, F), BF16),
            pltpu.VMEM((D, F), BF16),
            pltpu.VMEM((F, D), BF16),
            pltpu.VMEM((S, D), BF16),
            pltpu.SemaphoreType.DMA((12,)),
        ],
        compiler_params=pltpu.CompilerParams(vmem_limit_bytes=100 * 1024 * 1024),
        name="rmt_mod",
    )(A_x.reshape(S, D), A_mem0.reshape(M, D), A_Wq, A_Wk, A_Wv, A_Wo.reshape(H * Dh, D),
      B_w_r.reshape(D // 128, 128), B_w_gate, B_w_up, B_w_down)
    return out.reshape(1, S, D)
```

```python
import functools

import jax
import jax.numpy as jnp
import numpy as np
from jax import lax
import jax.experimental.pallas as pl
import jax.experimental.pallas.tpu as pltpu

F32 = jnp.float32
BF16 = jnp.bfloat16
U32 = jnp.uint32

_NN = (((1,), (0,)), ((), ()))
_NT = (((1,), (1,)), ((), ()))
_PRE = 8
_OUT_BLK = 8


def _rb(x):
    return x.astype(BF16).astype(F32)


def _layernorm(x):
    n = x.shape[-1]
    m = jnp.sum(x, axis=-1, keepdims=True) * (1.0 / n)
    xc = x - m
    v = jnp.sum(xc * xc, axis=-1, keepdims=True) * (1.0 / n)
    sd = _rb(jnp.sqrt(_rb(_rb(v) + 1e-5)))
    return _rb(_rb(x - _rb(m)) * (1.0 / sd))


def _mm(a, w_u32):
    return lax.dot_general(a, pltpu.bitcast(w_u32, BF16), _NN, preferred_element_type=F32)


def _kernel(x_hbm, mem_ref, wq_hbm, wk_hbm, wv_hbm, wo_hbm, wr_ref, wg_hbm, wu_hbm, wd_hbm,
            out_hbm,
            xa, xb, xn, xp, hs, att, osc, raw, wqkv, pre, wo_raw, wo, wg, wu, wd, ob, fix, sems, osem,
            *, n_heads, dh):
    n_seg, seg, D = x_hbm.shape
    S = n_seg * seg
    n_mem = mem_ref.shape[0]
    live = seg - _PRE
    L = seg + n_mem
    G = 4
    NG = n_heads // G
    scale = float(dh) ** -0.5
    w_hbm = (wk_hbm, wq_hbm, wv_hbm)
    NC = 6

    def w_copy(c):
        return pltpu.make_async_copy(w_hbm[c // 2].at[:, pl.ds(16 * (c % 2), 16), :], raw.at[c], sems.at[c])

    NQ = 4
    dq = D // NQ
    c0 = [pltpu.make_async_copy(wk_hbm.at[pl.ds(i * dq, dq), pl.ds(0, 16), :], raw.at[0, pl.ds(i * dq, dq)], sems.at[13 + i])
          for i in range(NQ)]
    cxb = pltpu.make_async_copy(x_hbm.at[:, pl.ds(live, _PRE), :], xb, sems.at[6])
    cxa = pltpu.make_async_copy(x_hbm.at[:, pl.ds(0, live), :], xa, sems.at[7])
    co = pltpu.make_async_copy(wo_hbm, wo_raw, sems.at[8])
    cf = [pltpu.make_async_copy(a, b, sems.at[9 + i]) for i, (a, b) in enumerate(((wg_hbm, wg), (wu_hbm, wu), (wd_hbm, wd)))]

    cxb.start()
    for c in c0:
        c.start()
    for c in range(1, NC):
        w_copy(c).start()
    cxa.start()
    co.start()

    def relayout(c, i, after=(None, None)):
        a = pltpu.bitcast(raw[c, pl.ds(i * 16, 16)], U32).reshape(8, 2, 8, dh)
        ev, od = a[:, 0], a[:, 1]
        rows = pl.ds(i * 8, 8) if isinstance(i, int) else pl.ds(pl.multiple_of(i * 8, 8), 8)
        for b in range(2):
            e, o = (ev, od) if after[b] is None else (ev | after[b], od | after[b])
            if b == 0:
                w = (e & np.uint32(0xFFFF)) | (o << 16)
            else:
                w = (e >> 16) | (o & np.uint32(0xFFFF0000))
            t = jnp.swapaxes(w, 0, 1)
            for j in range(8):
                col = (j % 2) * 256 + b * 128
                wqkv[c * 4 + j // 2, rows, col:col + 128] = t[j]

    cxb.wait()

    def ln_pre(i, _):
        v = xb[pl.ds(i * 8, 8)].astype(F32).reshape(8 * _PRE, D)
        xp[pl.ds(pl.multiple_of(i * 32, 32), 32), :] = pltpu.bitcast(_layernorm(v).astype(BF16), U32)
    lax.fori_loop(0, n_seg // 8, ln_pre, None)
    att[...] = jnp.zeros(att.shape, F32)

    for i in range(NQ):
        c0[i].wait()

        def rl0(t, _):
            relayout(0, 2 * t)
            relayout(0, 2 * t + 1)
        lax.fori_loop(i * dq // 32, (i + 1) * dq // 32, rl0, None)

    def pre_tile(c, t, n=0):
        g = c * 4 + t // 4
        cs = slice((t % 4) * 128, (t % 4 + 1) * 128)
        y = _mm(pltpu.bitcast(xp[...], BF16), wqkv[g, :, cs])
        pre[g, :, cs] = y
        z = pltpu.bitcast(att[0:8, 0:128], U32)
        return [pltpu.bitcast(y[i * 448 // n:i * 448 // n + 8], U32) & z for i in range(n)]

    def pro(c, _):
        for t in range(8):
            pre_tile(c, t)
        pltpu.make_async_copy(raw.at[c + 1], raw.at[c + 1], sems.at[c + 1]).wait()
        for t in range(8):
            z = pre_tile(c, 8 + t, 8)
            for i in range(4):
                relayout(c + 1, 4 * t + i, z[2 * i:2 * i + 2])
    lax.fori_loop(0, NC - 1, pro, None)

    cxa.wait()
    co.wait()
    for c in cf:
        c.start()
    z = [None] * 4
    for t in range(16):
        for i in range(4):
            s = t * 4 + i
            v = xa[s].astype(F32)
            if z[i] is not None:
                v = pltpu.bitcast(pltpu.bitcast(v, U32) | jnp.tile(z[i], (live // 8, D // 128)), F32)
            xn[s] = _layernorm(v)
        z = pre_tile(NC - 1, t, 4)
        for i in range(4):
            w = pltpu.bitcast(wo_raw[pl.ds(t * 256 + i * 64, 64), :], U32)
            wo[t // 2, pl.ds((t % 2) * 128 + i * 32, 32), :] = w | jnp.tile(z[i], (4, D // 128))

    def pos(i):
        return jnp.where(i < live, i + n_mem, jnp.where(i < live + n_mem, i - live, i))
    row = pos(lax.broadcasted_iota(jnp.int32, (L, L), 0))
    col = pos(lax.broadcasted_iota(jnp.int32, (L, L), 1))
    mask = (row < n_mem) | (row >= col)
    c_exp = scale * float(np.log2(np.e))
    neg = -1e9 / scale

    wr = wr_ref[...].astype(F32)
    wr = jnp.concatenate([wr[i:i + 1, :] for i in range(D // 128)], axis=1)
    sub = lax.broadcasted_iota(jnp.int32, (8, 128), 0)

    def post(s, valid, top):
        b1, i1, b2, i2 = top
        r = pl.ds(pl.multiple_of(s * seg, seg), seg)
        x = jnp.concatenate([xa[s].astype(F32), xb[s].astype(F32)], axis=0)
        h = _rb(x + _rb(att[...]))
        hs[r, :] = h
        hn = _layernorm(h)
        ob[r, :] = (h + hn).astype(BF16)
        rr = _rb(jnp.sum(hn * wr, axis=-1, keepdims=True))
        for j in range(seg // 8):
            val = jnp.where(valid, jnp.broadcast_to(rr[8 * j:8 * j + 8], (8, 128)), -jnp.inf)
            idx = sub + (s * seg + 8 * j)
            g1 = val > b1
            g2 = val > b2
            b2 = jnp.where(g1, b1, jnp.where(g2, val, b2))
            i2 = jnp.where(g1, i1, jnp.where(g2, idx, i2))
            b1 = jnp.where(g1, val, b1)
            i1 = jnp.where(g1, idx, i1)
        return b1, i1, b2, i2

    def step(s, carry):
        mem, top = carry
        h = jnp.concatenate([xn[s], mem], axis=0).astype(BF16)
        pr = pl.ds(pl.multiple_of(s * _PRE, _PRE), _PRE)
        k, q, v, p, l, o = {}, {}, {}, {}, {}, {}
        acc = {}

        def proj(i):
            return jnp.concatenate([_mm(h, wqkv[i]), pre[i, pr, :]], axis=0)

        def K(g):
            k[g] = proj(g)

        def Q(g):
            q[g] = proj(NG + g)

        def V(g):
            v[g] = proj(2 * NG + g)

        def Sc(g):
            for i in range(G):
                cs = slice(i * dh, (i + 1) * dh)
                sc = lax.dot_general(q[g][:, cs], k[g][:, cs].astype(BF16), _NT, preferred_element_type=F32)
                sc = jnp.where(mask, sc, neg)
                e = jnp.exp2((sc - jnp.max(sc, axis=-1, keepdims=True)) * c_exp)
                p[g, i] = e
                l[g, i] = jnp.sum(e, axis=-1, keepdims=True)

        def PV(g):
            for i in range(G):
                cs = slice(i * dh, (i + 1) * dh)
                t = lax.dot_general(p[g, i], v[g][:, cs].astype(BF16), _NN, preferred_element_type=F32)
                r = pl.reciprocal(l[g, i], approx=True)
                osc[g, :, cs] = t * (r * (2.0 - l[g, i] * r))

        def O(gs, n):
            cs = slice(n * 128, (n + 1) * 128)
            t = acc.get(n)
            for g in gs:
                u = _mm(osc[g], wo[g, :, cs])
                t = u if t is None else t + u
            acc[n] = t

        K(0)
        top = post(jnp.maximum(s - 1, 0), s > 0, top)
        Q(0); V(0)
        for g in range(1, NG):
            K(g); Sc(g - 1); Q(g); V(g); PV(g - 1)
        first, second = range(0, 5), range(5, NG)
        O(first, 0); Sc(NG - 1); O(first, 1); O(first, 2); PV(NG - 1); O(first, 3)
        for n in range(4):
            O(second, n)
        out = jnp.concatenate([acc[n] for n in range(4)], axis=1)
        att[0:live, :] = out[:live]
        att[live:seg, :] = out[live + n_mem:]
        return out[live:live + n_mem], top

    blk = _OUT_BLK * seg
    n_blk = n_seg // _OUT_BLK

    def out_copy(b):
        r = pl.ds(pl.multiple_of(b * blk, blk), blk)
        return pltpu.make_async_copy(ob.at[r], out_hbm.at[r], osem)

    def outer(b, carry):
        carry = lax.fori_loop(b * _OUT_BLK, (b + 1) * _OUT_BLK, step, carry)

        @pl.when(b > 0)
        def _():
            out_copy(b - 1).start()
        return carry

    ninf = jnp.full((8, 128), -jnp.inf, F32)
    _, top = lax.fori_loop(0, n_blk, outer, (mem_ref[...].astype(F32), (ninf, sub, ninf, sub + 8)))
    b1, i1, b2, i2 = post(n_seg - 1, True, top)
    out_copy(n_blk - 1).start()

    big = np.int32(1 << 30)
    m1 = jnp.max(b1, axis=0, keepdims=True)
    t1 = jnp.min(jnp.where(b1 == m1, i1, big), axis=0, keepdims=True)
    won = i1 == t1
    cb = jnp.where(won, b2, b1)
    ci = jnp.where(won, i2, i1)
    m2 = jnp.max(cb, axis=0, keepdims=True)
    t2 = jnp.min(jnp.where(cb == m2, ci, big), axis=0, keepdims=True)
    idx1 = jnp.clip(t1[0, 0], 0, S - 1)
    idx2 = jnp.clip(t2[0, 0], 0, S - 1)

    for c in cf:
        c.wait()
    base1 = pl.multiple_of((idx1 // 16) * 16, 16)
    base2 = pl.multiple_of((idx2 // 16) * 16, 16)
    h = jnp.concatenate([hs[pl.ds(base1, 16), :], hs[pl.ds(base2, 16), :]], axis=0)
    hn = _layernorm(h)
    hb = hn.astype(BF16)
    gt = _rb(jnp.dot(hb, wg[...], preferred_element_type=F32))
    up = _rb(jnp.dot(hb, wu[...], preferred_element_type=F32))
    a = _rb(gt * _rb(jax.nn.sigmoid(gt))) * up
    y = _rb(jnp.dot(a.astype(BF16), wd[...], preferred_element_type=F32))
    rr = _rb(jnp.sum(hn * wr, axis=-1, keepdims=True))
    y = _rb(y * _rb(jax.nn.sigmoid(rr)))
    ri = lax.broadcasted_iota(jnp.int32, (32, D), 0)
    gi = jnp.where(ri < 16, ri + base1, ri + (base2 - 16))
    sel = (gi == idx1) | (gi == idx2)
    fix[...] = (h + _rb(hn + jnp.where(sel, y, 0.0))).astype(BF16)
    pltpu.make_async_copy(ob, out_hbm, osem).wait()
    f1 = pltpu.make_async_copy(fix.at[pl.ds(0, 16)], out_hbm.at[pl.ds(base1, 16)], sems.at[0])
    f2 = pltpu.make_async_copy(fix.at[pl.ds(16, 16)], out_hbm.at[pl.ds(base2, 16)], sems.at[12])
    f1.start()

    @pl.when(base1 != base2)
    def _():
        f2.start()
        f2.wait()
    f1.wait()


@functools.partial(jax.jit, static_argnames=("A_seg_len",))
def pallas_sequential_preLN__memory_aug_recurrent_mem_tr__moe_arch_mod__prompt_kernel(
    A_x, A_mem0, A_Wq, A_Wk, A_Wv, A_Wo, A_seg_len, B_x, B_w_r, B_w_gate, B_w_up, B_w_down,
):
    del B_x
    _, S, D = A_x.shape
    _, H, Dh = A_Wq.shape
    M = A_mem0.shape[1]
    F = B_w_gate.shape[1]
    seg = int(A_seg_len)
    n_seg = S // seg
    any_spec = pl.BlockSpec(memory_space=pl.ANY)
    vmem_spec = pl.BlockSpec(memory_space=pltpu.VMEM)
    out = pl.pallas_call(
        functools.partial(_kernel, n_heads=H, dh=Dh),
        out_shape=jax.ShapeDtypeStruct((S, D), A_x.dtype),
        in_specs=[any_spec, vmem_spec, any_spec, any_spec, any_spec, any_spec, vmem_spec, any_spec, any_spec, any_spec],
        out_specs=any_spec,
        scratch_shapes=[
            pltpu.VMEM((n_seg, seg - _PRE, D), BF16),
            pltpu.VMEM((n_seg, _PRE, D), BF16),
            pltpu.VMEM((n_seg, seg - _PRE, D), F32),
            pltpu.VMEM((n_seg * _PRE // 2, D), U32),
            pltpu.VMEM((S, D), F32),
            pltpu.VMEM((seg, D), F32),
            pltpu.VMEM((H // 4, seg + M, 4 * Dh), F32),
            pltpu.VMEM((6, D, 16, Dh), BF16),
            pltpu.VMEM((3 * H // 4, D // 2, 4 * Dh), U32),
            pltpu.VMEM((3 * H // 4, n_seg * _PRE, 4 * Dh), F32),
            pltpu.VMEM((H * Dh, D), BF16),
            pltpu.VMEM((H // 4, 2 * Dh, D), U32),
            pltpu.VMEM((D, F), BF16),
            pltpu.VMEM((D, F), BF16),
            pltpu.VMEM((F, D), BF16),
            pltpu.VMEM((S, D), BF16),
            pltpu.VMEM((32, D), BF16),
            pltpu.SemaphoreType.DMA((17,)),
            pltpu.SemaphoreType.DMA,
        ],
        compiler_params=pltpu.CompilerParams(vmem_limit_bytes=110 * 1024 * 1024),
        name="rmt_mod",
    )(A_x.reshape(n_seg, seg, D), A_mem0.reshape(M, D), A_Wq, A_Wk, A_Wv, A_Wo.reshape(H * Dh, D),
      B_w_r.reshape(D // 128, 128), B_w_gate, B_w_up, B_w_down)
    return out.reshape(1, S, D)
```

```python
import functools


import jax
import jax.numpy as jnp
import numpy as np
from jax import lax
import jax.experimental.pallas as pl
import jax.experimental.pallas.tpu as pltpu

F32 = jnp.float32
BF16 = jnp.bfloat16
U32 = jnp.uint32

_NN = (((1,), (0,)), ((), ()))
_NT = (((1,), (1,)), ((), ()))
_PRE = 8
_BLK = 8
_CH = 16


def _rb(x):
    return x.astype(BF16).astype(F32)


def _layernorm(x):
    n = x.shape[-1]
    m = jnp.sum(x, axis=-1, keepdims=True) * (1.0 / n)
    xc = x - m
    v = jnp.sum(xc * xc, axis=-1, keepdims=True) * (1.0 / n)
    sd = _rb(jnp.sqrt(_rb(_rb(v) + 1e-5)))
    return _rb(_rb(x - _rb(m)) * (1.0 / sd))


def _mm(a, w_u32):
    return lax.dot_general(a, pltpu.bitcast(w_u32, BF16), _NN, preferred_element_type=F32)


def _rows(start, size):
    return pl.ds(start, size) if isinstance(start, int) else pl.ds(pl.multiple_of(start, size), size)


def _kernel(x_hbm, mem_hbm, wq_hbm, wk_hbm, wv_hbm, wo_hbm, wr_hbm, wg_hbm, wu_hbm, wd_hbm,
            out_hbm,
            mem_ref, wr_ref, xa, xb, xn, xp, hs, att, zero, osc, raw, wqkv, pre, wo_raw, wo, wg, wu, wd, ob, fix, sems, osem):
    n_seg, seg, D = x_hbm.shape
    _, H, dh = wq_hbm.shape
    S = n_seg * seg
    n_mem = mem_ref.shape[0]
    live = seg - _PRE
    L = seg + n_mem
    G = 4
    NG = H // G
    scale = float(dh) ** -0.5
    w_hbm = (wk_hbm, wq_hbm, wv_hbm)
    NC = 3 * H // _CH

    def w_copy(c):
        return pltpu.make_async_copy(w_hbm[c // 2].at[:, pl.ds(_CH * (c % 2), _CH), :], raw.at[c], sems.at[c])

    NQ = 4
    dq = D // NQ
    c0 = [pltpu.make_async_copy(wk_hbm.at[pl.ds(i * dq, dq), pl.ds(0, _CH), :], raw.at[0, pl.ds(i * dq, dq)], sems.at[13 + i])
          for i in range(NQ)]
    cxb = pltpu.make_async_copy(x_hbm.at[:, pl.ds(live, _PRE), :], xb, sems.at[6])
    NB = NC - 2

    def xa_copy(c):
        r = pl.ds(c * (n_seg // NB), n_seg // NB)
        return pltpu.make_async_copy(x_hbm.at[r, pl.ds(0, live), :], xa.at[r], sems.at[17 + c])

    def wo_copy(c):
        r = pl.ds(c * (NG // NB), NG // NB)
        return pltpu.make_async_copy(wo_hbm.at[r], wo_raw.at[r], sems.at[21 + c])

    cf = [pltpu.make_async_copy(a, b, sems.at[9 + i]) for i, (a, b) in enumerate(((wg_hbm, wg), (wu_hbm, wu), (wd_hbm, wd)))]

    cxb.start()
    for c in c0:
        c.start()
    for c in range(1, NC):
        w_copy(c).start()
    small = [pltpu.make_async_copy(mem_hbm, mem_ref, sems.at[7]), pltpu.make_async_copy(wr_hbm, wr_ref, sems.at[8])]
    for c in small:
        c.start()
    for c in range(NB):
        xa_copy(c).start()
        wo_copy(c).start()

    def relayout(c, i, after=(None, None)):
        a = pltpu.bitcast(raw[c, pl.ds(i * 16, 16)], U32).reshape(8, 2, _CH // 2, dh)
        ev, od = a[:, 0], a[:, 1]
        for b in range(2):
            e, o = (ev, od) if after[b] is None else (ev | after[b], od | after[b])
            if b == 0:
                w = (e & np.uint32(0xFFFF)) | (o << 16)
            else:
                w = (e >> 16) | (o & np.uint32(0xFFFF0000))
            t = jnp.swapaxes(w, 0, 1)
            for j in range(_CH // 2):
                wqkv[c * _CH + 2 * j + b, _rows(i * 8, 8), :] = t[j]

    cxb.wait()

    def ln_pre(i, _):
        v = xb[pl.ds(i * 32, 32)].astype(F32).reshape(32 * _PRE, D)
        xp[_rows(i * 128, 128), :] = pltpu.bitcast(_layernorm(v).astype(BF16), U32)
    lax.fori_loop(0, n_seg // 32, ln_pre, None)
    att[...] = jnp.zeros(att.shape, F32)
    zero[...] = jnp.zeros(zero.shape, U32)

    for i in range(NQ):
        c0[i].wait()

        def rl0(t, _):
            relayout(0, 2 * t)
            relayout(0, 2 * t + 1)
        lax.fori_loop(i * dq // 32, (i + 1) * dq // 32, rl0, None)

    def pre_tile(t, n=0):
        y = _mm(pltpu.bitcast(xp[...], BF16), wqkv[t])
        pre[t] = y
        z = zero[...]
        return [pltpu.bitcast(y[i * 448 // n:i * 448 // n + 8], U32) & z for i in range(n)]

    def pre_block(t, b):
        r = _BLK * _PRE
        pre[t, _rows(b * r, r), :] = _mm(pltpu.bitcast(xp[_rows(b * (r // 2), r // 2), :], BF16), wqkv[t])

    n_fill = _CH
    n_pro = 3 * H - n_fill
    for t in range(8):
        pre_tile(t)

    def pro_a(c, _):
        pltpu.make_async_copy(raw.at[c], raw.at[c], sems.at[c]).wait()
        for t in range(8):
            z = pre_tile(c * _CH + (t - 8), 8)
            for i in range(4):
                relayout(c, 4 * t + i, z[2 * i:2 * i + 2])
    lax.fori_loop(1, NC, pro_a, None)
    for c in small:
        c.wait()

    def pro_b(c, _):
        xa_copy(c).wait()
        wo_copy(c).wait()
        z = [None] * 4
        for t in range(8):
            for i in range(2):
                s = c * (n_seg // NB) + (t * 2 + i)
                v = xa[s].astype(F32)
                if z[i] is not None:
                    v = pltpu.bitcast(pltpu.bitcast(v, U32) | jnp.tile(z[i], (live // 8, D // 128)), F32)
                xn[s] = _layernorm(v)
            z = pre_tile((c + 1) * _CH + t, 4)
            for i in range(2):
                j = (t % 4) * 2 + i
                w = pltpu.bitcast(wo_raw[c * 2 + t // 4, pl.ds(j * 64, 64), :], U32)
                wo[c * 2 + t // 4, pl.ds(j * 32, 32), :] = w | jnp.tile(z[2 + i], (4, D // 128))
    lax.fori_loop(0, NB, pro_b, None)

    for t in range(n_pro, 3 * H):
        pre_block(t, 0)

    def pos(i):
        return jnp.where(i < live, i + n_mem, jnp.where(i < live + n_mem, i - live, i))
    row = pos(lax.broadcasted_iota(jnp.int32, (L, L), 0))
    col = pos(lax.broadcasted_iota(jnp.int32, (L, L), 1))
    mask = (row < n_mem) | (row >= col)
    c_exp = scale * float(np.log2(np.e))
    neg = -1e9 / scale

    wr = wr_ref[...].astype(F32)
    wr = jnp.concatenate([wr[i:i + 1, :] for i in range(D // 128)], axis=1)
    sub = lax.broadcasted_iota(jnp.int32, (8, 128), 0)

    def post(s, half, valid, top):
        b1, i1, b2, i2 = top
        r = _rows(s * seg + half * 16, 16)
        if half == 0:
            x = xa[s, 0:16].astype(F32)
        else:
            x = jnp.concatenate([xa[s, 16:live].astype(F32), xb[s].astype(F32)], axis=0)
        h = _rb(x + _rb(att[half * 16:half * 16 + 16]))
        hs[r, :] = h
        hn = _layernorm(h)
        ob[r, :] = (h + hn).astype(BF16)
        rr = _rb(jnp.sum(hn * wr, axis=-1, keepdims=True))
        for j in range(2):
            val = jnp.broadcast_to(rr[8 * j:8 * j + 8], (8, 128))
            if valid is not None:
                val = jnp.where(valid, val, -jnp.inf)
            idx = sub + (s * seg + half * 16 + 8 * j)
            g1 = val > b1
            g2 = val > b2
            b2 = jnp.where(g1, b1, jnp.where(g2, val, b2))
            i2 = jnp.where(g1, i1, jnp.where(g2, idx, i2))
            b1 = jnp.where(g1, val, b1)
            i1 = jnp.where(g1, idx, i1)
        return b1, i1, b2, i2

    def step(s, first_in_block, carry):
        mem, top = carry
        h = jnp.concatenate([xn[s], mem], axis=0).astype(BF16)
        pr = _rows(s * _PRE, _PRE)
        k, q, v, p = {}, {}, {}, {}
        before = {}
        acc = {}

        def proj(dst, m, g):
            for i in range(g * G, (g + 1) * G):
                ahead = pre[m * H + i, pr, :]
                if (m, i) in before:
                    ahead = pltpu.bitcast(pltpu.bitcast(ahead, U32) | (before[m, i] & zero[...]), F32)
                dst[i] = jnp.concatenate([_mm(h, wqkv[m * H + i]), ahead], axis=0)

        def K(g):
            proj(k, 0, g)

        def Q(g):
            proj(q, 1, g)

        def V(g):
            proj(v, 2, g)

        def Sc(g):
            for i in range(g * G, (g + 1) * G):
                sc = lax.dot_general(q[i], k[i].astype(BF16), _NT, preferred_element_type=F32)
                sc = jnp.where(mask, sc, neg)
                e = jnp.exp2((sc - jnp.max(sc, axis=-1, keepdims=True)) * c_exp)
                l = jnp.sum(e, axis=-1, keepdims=True)
                r = pl.reciprocal(l, approx=True)
                p[i] = e * (r * (2.0 - l * r))

        def PV(g):
            for i in range(g * G, (g + 1) * G):
                t = lax.dot_general(p[i], v[i].astype(BF16), _NN, preferred_element_type=F32)
                osc[g, :, pl.ds((i % G) * dh, dh)] = jnp.concatenate([t[live:live + n_mem], t[:live], t[live + n_mem:]], axis=0)

        def O(gs, n):
            cs = slice(n * 128, (n + 1) * 128)
            t = acc.get(n)
            for g in gs:
                u = _mm(osc[g], wo[g, :, cs])
                t = u if t is None else t + u
            acc[n] = t

        prev, valid = (jnp.maximum(s - 1, 0), s > 0) if first_in_block else (s - 1, None)
        for half in range(2):
            top = post(prev, half, valid, top)
            before[1, (1 + half) * G] = pltpu.bitcast(top[3], U32)
        K(0); Q(0); V(0)
        for g in range(1, NG):
            K(g); Sc(g - 1); Q(g)
            if g > 1:
                PV(g - 2)
            V(g)
        first, second = range(0, 5), range(5, NG)
        O(first, 0); Sc(NG - 1); O(first, 1); PV(NG - 2); O(first, 2); O(first[:2], 3); PV(NG - 1); O(first[2:], 3)
        for n in range(4):
            O(second, n)
        out = jnp.concatenate([acc[n] for n in range(4)], axis=1)
        att[...] = out[n_mem:]
        return out[:n_mem], top

    blk = _BLK * seg
    n_blk = n_seg // _BLK

    def out_copy(b):
        r = _rows(b * blk, blk)
        return pltpu.make_async_copy(ob.at[r], out_hbm.at[r], osem)

    def steps(b, carry):
        nxt = jnp.where(b + 1 < n_blk, b + 1, 0)
        for u in range(_BLK):
            carry = step(b * _BLK + u, u == 0, carry)
            if u + 1 < _BLK:
                for t in range(n_fill * u // (_BLK - 1), n_fill * (u + 1) // (_BLK - 1)):
                    pre_block(n_pro + t, nxt)

        @pl.when(b > 0)
        def _():
            out_copy(b - 1).start()

        @pl.when(b == 1)
        def _():
            for c in cf:
                c.start()
        return carry

    ninf = jnp.full((8, 128), -jnp.inf, F32)
    _, top = lax.fori_loop(0, n_blk, steps, (mem_ref[...].astype(F32), (ninf, sub, ninf, sub + 8)))
    for c in cf:
        c.wait()
    b1, i1, b2, i2 = post(n_seg - 1, 1, None, post(n_seg - 1, 0, None, top))
    out_copy(n_blk - 1).start()

    big = np.int32(1 << 30)
    m1 = jnp.max(b1, axis=0, keepdims=True)
    t1 = jnp.min(jnp.where(b1 == m1, i1, big), axis=0, keepdims=True)
    won = i1 == t1
    cb = jnp.where(won, b2, b1)
    ci = jnp.where(won, i2, i1)
    m2 = jnp.max(cb, axis=0, keepdims=True)
    t2 = jnp.min(jnp.where(cb == m2, ci, big), axis=0, keepdims=True)
    idx1 = jnp.clip(t1[0, 0], 0, S - 1)
    idx2 = jnp.clip(t2[0, 0], 0, S - 1)

    base1 = pl.multiple_of((idx1 // 16) * 16, 16)
    base2 = pl.multiple_of((idx2 // 16) * 16, 16)
    h = jnp.concatenate([hs[pl.ds(base1, 16), :], hs[pl.ds(base2, 16), :]], axis=0)
    hn = _layernorm(h)
    hb = hn.astype(BF16)
    gt = _rb(jnp.dot(hb, wg[...], preferred_element_type=F32))
    up = _rb(jnp.dot(hb, wu[...], preferred_element_type=F32))
    a = _rb(gt * _rb(jax.nn.sigmoid(gt))) * up
    y = _rb(jnp.dot(a.astype(BF16), wd[...], preferred_element_type=F32))
    rr = _rb(jnp.sum(hn * wr, axis=-1, keepdims=True))
    y = _rb(y * _rb(jax.nn.sigmoid(rr)))
    ri = lax.broadcasted_iota(jnp.int32, (32, D), 0)
    gi = jnp.where(ri < 16, ri + base1, ri + (base2 - 16))
    sel = (gi == idx1) | (gi == idx2)
    fix[...] = (h + _rb(hn + jnp.where(sel, y, 0.0))).astype(BF16)
    pltpu.make_async_copy(ob, out_hbm, osem).wait()
    f1 = pltpu.make_async_copy(fix.at[pl.ds(0, 16)], out_hbm.at[pl.ds(base1, 16)], sems.at[0])
    f2 = pltpu.make_async_copy(fix.at[pl.ds(16, 16)], out_hbm.at[pl.ds(base2, 16)], sems.at[12])
    f1.start()

    @pl.when(base1 != base2)
    def _():
        f2.start()
        f2.wait()
    f1.wait()


@functools.partial(jax.jit, static_argnames=("A_seg_len",))
def pallas_sequential_preLN__memory_aug_recurrent_mem_tr__moe_arch_mod__prompt_kernel(
    A_x, A_mem0, A_Wq, A_Wk, A_Wv, A_Wo, A_seg_len, B_x, B_w_r, B_w_gate, B_w_up, B_w_down,
):
    del B_x
    _, S, D = A_x.shape
    _, H, Dh = A_Wq.shape
    M = A_mem0.shape[1]
    F = B_w_gate.shape[1]
    seg = int(A_seg_len)
    n_seg = S // seg
    any_spec = pl.BlockSpec(memory_space=pl.ANY)
    vmem_spec = pl.BlockSpec(memory_space=pltpu.VMEM)
    out = pl.pallas_call(
        _kernel,
        out_shape=jax.ShapeDtypeStruct((S, D), A_x.dtype),
        in_specs=[any_spec] * 10,
        out_specs=any_spec,
        scratch_shapes=[
            pltpu.VMEM((M, D), BF16),
            pltpu.VMEM((D // 128, 128), BF16),
            pltpu.VMEM((n_seg, seg - _PRE, D), BF16),
            pltpu.VMEM((n_seg, _PRE, D), BF16),
            pltpu.VMEM((n_seg, seg - _PRE, D), F32),
            pltpu.VMEM((n_seg * _PRE // 2, D), U32),
            pltpu.VMEM((S, D), F32),
            pltpu.VMEM((seg, D), F32),
            pltpu.VMEM((8, 128), U32),
            pltpu.VMEM((H // 4, seg + M, 4 * Dh), F32),
            pltpu.VMEM((3 * H // _CH, D, _CH, Dh), BF16),
            pltpu.VMEM((3 * H, D // 2, Dh), U32),
            pltpu.VMEM((3 * H, n_seg * _PRE, Dh), F32),
            pltpu.VMEM((H // 4, 4 * Dh, D), BF16),
            pltpu.VMEM((H // 4, 2 * Dh, D), U32),
            pltpu.VMEM((D, F), BF16),
            pltpu.VMEM((D, F), BF16),
            pltpu.VMEM((F, D), BF16),
            pltpu.VMEM((S, D), BF16),
            pltpu.VMEM((32, D), BF16),
            pltpu.SemaphoreType.DMA((25,)),
            pltpu.SemaphoreType.DMA,
        ],
        compiler_params=pltpu.CompilerParams(vmem_limit_bytes=110 * 1024 * 1024),
        name="rmt_mod",
    )(A_x.reshape(n_seg, seg, D), A_mem0.reshape(M, D), A_Wq, A_Wk, A_Wv, A_Wo.reshape(H // 4, 4 * Dh, D),
      B_w_r.reshape(D // 128, 128), B_w_gate, B_w_up, B_w_down)
    return out.reshape(1, S, D)
```

```python
import functools

import jax
import jax.numpy as jnp
import numpy as np
from jax import lax
import jax.experimental.pallas as pl
import jax.experimental.pallas.tpu as pltpu

F32 = jnp.float32
BF16 = jnp.bfloat16
U32 = jnp.uint32

_NN = (((1,), (0,)), ((), ()))
_NT = (((1,), (1,)), ((), ()))
_PRE = 8
_BLK = 8
_CH = 16


def _rb(x):
    return x.astype(BF16).astype(F32)


def _layernorm(x):
    n = x.shape[-1]
    m = jnp.sum(x, axis=-1, keepdims=True) * (1.0 / n)
    xc = x - m
    v = jnp.sum(xc * xc, axis=-1, keepdims=True) * (1.0 / n)
    sd = _rb(jnp.sqrt(_rb(_rb(v) + 1e-5)))
    return _rb(_rb(x - _rb(m)) * (1.0 / sd))


def _mm(a, w_u32):
    return lax.dot_general(a, pltpu.bitcast(w_u32, BF16), _NN, preferred_element_type=F32)


def _forms(b11, b12, b21, b22):
    f11, f12, f21, f22 = (b.astype(F32) for b in (b11, b12, b21, b22))
    return ((f11 + f22).astype(BF16), b11, (f12 - f22).astype(BF16), (f21 - f11).astype(BF16), b22,
            (f11 + f12).astype(BF16), (f21 + f22).astype(BF16))


def _swap8(w):
    sub = lax.broadcasted_iota(jnp.int32, w[0].shape, 0)
    u = [pltpu.roll(w[-k % 8], -k % 8, 0) if k else w[0] for k in range(8)]
    for b in (1, 2, 4):
        u = [jnp.where((sub & b) != 0, u[(k - b) % 8], u[k]) for k in range(8)]
    return [pltpu.roll(u[j], -j % 8, 0) if j else u[0] for j in range(8)]


def _rows(start, size):
    return pl.ds(start, size) if isinstance(start, int) else pl.ds(pl.multiple_of(start, size), size)


def _kernel(x_hbm, mem_hbm, wq_hbm, wk_hbm, wv_hbm, wo_hbm, wr_hbm, wg_hbm, wu_hbm, wd_hbm,
            out_hbm,
            mem_ref, wr_ref, xa, xb, xn, xp, hs, att, zero, osc, osm, a12, raw, wqkv, wf, part, nxt, gam, pre, wo_raw, wo, wg, wu, wd, ob, fix, sems, osem):
    n_seg, seg, D = x_hbm.shape
    _, H, dh = wq_hbm.shape
    S = n_seg * seg
    n_mem = mem_ref.shape[0]
    live = seg - _PRE
    L = seg + n_mem
    G = 4
    NG = H // G
    scale = float(dh) ** -0.5
    w_hbm = (wk_hbm, wq_hbm, wv_hbm)
    NC = 3 * H // _CH

    def w_copy(c):
        return pltpu.make_async_copy(w_hbm[c // 2].at[:, pl.ds(_CH * (c % 2), _CH), :], raw.at[c], sems.at[c])

    NQ = 4
    dq = D // NQ
    c0 = [pltpu.make_async_copy(wk_hbm.at[pl.ds(i * dq, dq), pl.ds(0, _CH), :], raw.at[0, pl.ds(i * dq, dq)], sems.at[13 + i])
          for i in range(NQ)]
    cxb = pltpu.make_async_copy(x_hbm.at[:, pl.ds(live, _PRE), :], xb, sems.at[6])
    NB = NC - 2

    n_early = 2 * _BLK
    cxa = [pltpu.make_async_copy(x_hbm.at[r, pl.ds(0, live), :], xa.at[r], sems.at[17 + i])
           for i, r in enumerate((pl.ds(0, 2), pl.ds(2, n_early - 2), pl.ds(n_early, n_seg - n_early)))]

    def wo_copy(c):
        r = pl.ds(c * (H // NB), H // NB)
        return pltpu.make_async_copy(wo_hbm.at[r], wo_raw.at[r], sems.at[21 + c])

    cf = [pltpu.make_async_copy(a, b, sems.at[9 + i]) for i, (a, b) in enumerate(((wg_hbm, wg), (wu_hbm, wu), (wd_hbm, wd)))]

    cxb.start()
    cxa[0].start()
    for c in c0:
        c.start()
    for c in range(1, NC):
        w_copy(c).start()
    small = [pltpu.make_async_copy(mem_hbm, mem_ref, sems.at[7]), pltpu.make_async_copy(wr_hbm, wr_ref, sems.at[8])]
    for c in small:
        c.start()
    for c in range(NB):
        wo_copy(c).start()
    cxa[1].start()
    cxa[2].start()

    def relayout(c, i, after=(None, None)):
        a = pltpu.bitcast(raw[c, pl.ds(i * 16, 16)], U32).reshape(8, 2, _CH // 2, dh)
        ev, od = a[:, 0], a[:, 1]
        for b in range(2):
            e, o = (ev, od) if after[b] is None else (ev | after[b], od | after[b])
            if b == 0:
                w = (e & np.uint32(0xFFFF)) | (o << 16)
            else:
                w = (e >> 16) | (o & np.uint32(0xFFFF0000))
            t = _swap8([w[j] for j in range(8)])
            for j in range(_CH // 2):
                wqkv[c * _CH + 2 * j + b, _rows(i * 8, 8), :] = t[j]

    cxb.wait()
    cxa[0].wait()

    def ln_pre(i, _):
        v = xb[pl.ds(i * 32, 32)].astype(F32).reshape(32 * _PRE, D)
        xp[_rows(i * 128, 128), :] = pltpu.bitcast(_layernorm(v).astype(BF16), U32)
    lax.fori_loop(0, n_seg // 32, ln_pre, None)
    zero[...] = jnp.zeros(zero.shape, U32)

    for i in range(NQ):
        c0[i].wait()

        def rl0(t, _):
            relayout(0, 2 * t)
            relayout(0, 2 * t + 1)
        lax.fori_loop(i * dq // 32, (i + 1) * dq // 32, rl0, None)

    half = D // 2

    def pace(y, n):
        return [pltpu.bitcast(y[r:r + 8], U32) & zero[...] for r in (i * 60 // n * 8 for i in range(n))]

    def pre_tile(t, first, r0, r):
        k0 = half if first else 0
        y = _mm(pltpu.bitcast(xp[_rows(r0 // 2, r // 2), k0:], BF16), wqkv[t, k0 // 2:])
        pre[t, _rows(r0, r), :] = y
        return y

    def token_forms(job, j):
        r = pl.ds(j * 8, 8)
        top, bot = (_layernorm(xa[2 * job + i, r].astype(F32)) for i in range(2))
        a11, a12_, a21, a22 = top[:, :half], top[:, half:], bot[:, :half], bot[:, half:]
        fs = (a11 + a22, a21 + a22, a11, a22, a11 + a12_, a21 - a11, a12_ - a22)
        for f, v in enumerate(fs):
            xn[f, r, :] = v
        return fs[0][:, :128]

    def w_form(f, pair):
        if f == 1:
            return wqkv[2 * pair, :half // 2]
        if f == 4:
            return wqkv[2 * pair + 1, half // 2:]
        return wf[(0, None, 1, 2, None, 3, 4)[f], pair]

    def ahead_products(pair, lhs):
        m1, m6, m7, mg = (_mm(lhs[f], w_form(f, pair)) for f in (0, 5, 6, 1))
        part[2 * pair] = (m1 + m7)[:live]
        part[2 * pair + 1] = (m1 + m6)[:live]
        gam[pair] = mg[:2 * _PRE]
        return m1, m6, m7, mg

    n_ahead = n_seg * _PRE
    n_pro = 3 * H - _CH
    fill = [(n_pro + 2 * j + 1, False) for j in range(_CH // 2)] + [(n_pro + 2 * j, True) for j in range(_CH // 2)]
    att[...] = jnp.zeros(att.shape, F32)
    for f in (0, 1, 5, 6):
        osc[f] = jnp.zeros(osc.shape[1:], F32)
    for j in range(live // 8):
        token_forms(0, j)
    for j in range(_CH // 2):
        pre_tile(2 * j, True, 0, n_ahead)

    def qkv_forms(pair, j, after):
        r = (pl.ds(j * 16, 16), pl.ds(half // 2 + j * 16, 16))
        w = [wqkv[2 * pair + b, r[a]] for a in range(2) for b in range(2)]
        if after is not None:
            w = [x | jnp.tile(after, (2, 1)) for x in w]
        fs = _forms(*(pltpu.bitcast(x, BF16) for x in w))
        for i, f in enumerate((0, 2, 3, 5, 6)):
            wf[i, pair, r[0]] = pltpu.bitcast(fs[f], U32)

    def pro_a(c, _):
        pltpu.make_async_copy(raw.at[c], raw.at[c], sems.at[c]).wait()
        for t in range(8):
            z = pace(pre_tile(c * _CH + (2 * t + 1 - _CH), False, 0, n_ahead), 16)
            for i in range(4):
                relayout(c, 4 * t + i, z[4 * i:4 * i + 2])
                qkv_forms(c * 8 + (t - 8), 2 * i, z[4 * i + 2])
                qkv_forms(c * 8 + (t - 8), 2 * i + 1, z[4 * i + 3])
    lax.fori_loop(1, NC, pro_a, None)
    for c in small:
        c.wait()

    def wo_forms(c, pair, j, after):
        def rows(head):
            w = pltpu.bitcast(wo_raw[c * 8 + 2 * pair + head, pl.ds(j * 16, 16), :], U32)
            w = pltpu.bitcast(w | jnp.tile(after, (1, D // 128)), BF16)
            return w[:, :D // 2], w[:, D // 2:]
        for f, w in enumerate(_forms(*rows(0), *rows(1))):
            wo[f, c, pl.ds(pair * (dh // 2) + j * 8, 8), :] = pltpu.bitcast(w, U32)

    def pro_b(c, _):
        wo_copy(c).wait()
        z = []
        for t in range(_CH // 2):
            y = pre_tile((c + 1) * _CH + 2 * t, True, 0, n_ahead)
            if t % 2:
                z += pace(y, 12)
        for i in range(16):
            qkv_forms(n_pro // 2 + c * 2 + i // 8, i % 8, z[i])
        for i in range(32):
            wo_forms(c, i // 8, i % 8, z[16 + i])
        lhs = {f: xn[f].astype(BF16) for f in (0, 5, 6)}
        lhs[1] = pltpu.bitcast(xp[0:_PRE, :half], BF16)
        for i in range(2 * NC):
            ahead_products(c * 2 + (i // 2 * 8 + i % 2), lhs)
        for i in range(4):
            pre_tile(n_pro + c * 4 + (1, 3, 0, 2)[i], i > 1, 0, _BLK * _PRE)
    lax.fori_loop(0, NB, pro_b, None)
    cxa[1].wait()

    def pos(i):
        return jnp.where(i < live, i + n_mem, jnp.where(i < live + n_mem, i - live, i))
    row = pos(lax.broadcasted_iota(jnp.int32, (L, L), 0))
    col = pos(lax.broadcasted_iota(jnp.int32, (L, L), 1))
    mask = (row < n_mem) | (row >= col)
    c_exp = scale * float(np.log2(np.e))
    neg = -1e9 / scale

    wr = wr_ref[...].astype(F32)
    wr = jnp.concatenate([wr[i:i + 1, :] for i in range(D // 128)], axis=1)
    sub = lax.broadcasted_iota(jnp.int32, (8, 128), 0)

    def post(s, part_, valid, top, at):
        b1, i1, b2, i2 = top
        r = _rows(s * seg + part_ * 16, 16)
        if part_ == 0:
            x = xa[s, 0:16].astype(F32)
        else:
            x = jnp.concatenate([xa[s, 16:live].astype(F32), xb[s].astype(F32)], axis=0)
        h = _rb(x + _rb(att[at + part_ * 16:at + part_ * 16 + 16]))
        hs[r, :] = h
        hn = _layernorm(h)
        ob[r, :] = (h + hn).astype(BF16)
        rr = _rb(jnp.sum(hn * wr, axis=-1, keepdims=True))
        for j in range(2):
            val = jnp.broadcast_to(rr[8 * j:8 * j + 8], (8, 128))
            if valid is not None:
                val = jnp.where(valid, val, -jnp.inf)
            idx = sub + (s * seg + part_ * 16 + 8 * j)
            g1 = val > b1
            g2 = val > b2
            b2 = jnp.where(g1, b1, jnp.where(g2, val, b2))
            i2 = jnp.where(g1, i1, jnp.where(g2, idx, i2))
            b1 = jnp.where(g1, val, b1)
            i1 = jnp.where(g1, idx, i1)
        return b1, i1, b2, i2

    o_plan = (((0, 0, seg, 1), (5, 0, seg, 0), (6, 0, seg, 1), (1, seg // 2, seg, 2)),
              ((3, 0, seg, 1), (2, 0, seg, 0), (4, 0, seg, 2), (1, 0, seg // 2, 2)))

    def o_tokens(odd, n, r):
        lo, hi = pl.ds(n * 128, 128), pl.ds(D // 2 + n * 128, 128)
        hs_ = seg // 2
        if odd:
            m4, m3, m5, m2 = r
            att[0:seg, lo] = m4 - m5
            att[0:seg, hi] = m3 + m5
            att[seg:seg + hs_, lo] = m4[:hs_] + m2
            att[seg + hs_:2 * seg, lo] = m4[hs_:]
            att[seg:seg + hs_, hi] = m3[:hs_] - m2
            att[seg + hs_:2 * seg, hi] = m3[hs_:]
        else:
            m1, m6, m7, m2 = r
            att[0:seg, lo] += m1 + m7
            att[seg + hs_:2 * seg, lo] += m2
            t = m1 + m6
            att[seg:seg + hs_, hi] += t[:hs_]
            att[seg + hs_:2 * seg, hi] += t[hs_:] - m2

    def step(s, u, carry):
        odd = u % 2
        mem, top = carry
        a1, a2 = mem[:, :half], mem[:, half:]
        a3 = a1 + a2
        if odd:
            job = jnp.where(s + 1 < n_seg, (s + 1) // 2, 0) if u + 1 == _BLK else (s + 1) // 2
            lhs = {f: jnp.concatenate([xn[f], a], axis=0).astype(BF16) for f, a in ((0, a2), (5, a1), (6, a2))}
            lhs[1] = jnp.concatenate([pltpu.bitcast(xp[_rows(job * _PRE, _PRE), :half], BF16), a3.astype(BF16)], axis=0)
        else:
            lhs = {f: jnp.concatenate([xn[f], a], axis=0).astype(BF16) for f, a in ((1, a3), (2, a1), (3, a2), (4, a3))}
        pr = _rows(s * _PRE, _PRE)
        k, q, v, p = {}, {}, {}, {}
        before = {}
        acc = {}

        def proj(dst, m, g):
            for i in range(g * G, (g + 1) * G, 2):
                t = m * H + i
                ahead = [pre[t, pr, :] + gam[t // 2, pl.ds(odd * _PRE, _PRE)], pre[t + 1, pr, :]]
                if (m, i) in before:
                    ahead[1] = pltpu.bitcast(pltpu.bitcast(ahead[1], U32) | (before[m, i] & zero[...]), F32)
                if odd:
                    m1, m6, m7, mg = ahead_products(t // 2, lhs)
                    d = mg[2 * _PRE:] - m1[live:]
                    dst[i] = jnp.concatenate([nxt[t], m7[live:] + d, ahead[0]], axis=0)
                    dst[i + 1] = jnp.concatenate([nxt[t + 1], m6[live:] - d, ahead[1]], axis=0)
                else:
                    m2, m4, m3, m5 = (_mm(lhs[f], w_form(f, t // 2)) for f in (1, 3, 2, 4))
                    y = m2 + m4
                    nxt[t] = y[:live]
                    nxt[t + 1] = part[t + 1] + (m3 - m2)[:live]
                    dst[i] = jnp.concatenate([part[t] + (m4 - m5)[:live], y[live:], ahead[0]], axis=0)
                    dst[i + 1] = jnp.concatenate([m3 + m5, ahead[1]], axis=0)

        def K(g):
            proj(k, 0, g)

        def Q(g):
            proj(q, 1, g)

        def V(g):
            proj(v, 2, g)

        def Sc(g):
            for i in range(g * G, (g + 1) * G):
                sc = lax.dot_general(q[i], k[i].astype(BF16), _NT, preferred_element_type=F32)
                sc = jnp.where(mask, sc, neg)
                e = jnp.exp2((sc - jnp.max(sc, axis=-1, keepdims=True)) * c_exp)
                l = jnp.sum(e, axis=-1, keepdims=True)
                r = pl.reciprocal(l, approx=True)
                p[i] = e * (r * (2.0 - l * r))

        def PV(g):
            o = [lax.dot_general(p[i], v[i].astype(BF16), _NN, preferred_element_type=F32)
                 for i in range(g * G, (g + 1) * G)]
            for j in range(G // 2):
                t = g * (G // 2) + j
                c, cs = t // 4, pl.ds((t % 4) * dh, dh)
                m1, m2 = (x[live:live + n_mem] for x in o[2 * j:2 * j + 2])
                osm[0, c, :, cs] = m1
                osm[1, c, :, cs] = m2
                osm[2, c, :, cs] = m1 + m2
                x1, x2 = (jnp.concatenate([x[:live], x[live + n_mem:]], axis=0) for x in o[2 * j:2 * j + 2])
                if odd:
                    y1, y2 = osc[2, c, :, cs], a12[t]
                    osc[3, c, :, cs] = x2
                    osc[1, c, :, cs] = x1 + x2
                    osc[0, c, :, cs] = y1 + x2
                    osc[5, c, :, cs] = x1 - y1
                    osc[6, c, :, cs] = y2 - x2
                else:
                    osc[2, c, :, cs] = x1
                    osc[4, c, :, cs] = x1 + x2
                    a12[t] = x2

        def O(cs_, n, j):
            f, r0, r1, fm = o_plan[odd][j]
            t = acc.get((n, j))
            for c in cs_:
                lhs = jnp.concatenate([osm[fm, c], osc[f, c, r0:r1]], axis=0)
                y = _mm(lhs, wo[f, c, :, n * 128:(n + 1) * 128])
                t = y if t is None else t + y
            acc[n, j] = t

        if odd:
            base, valid = (jnp.maximum(s - 3, 0), s > 1) if u == 1 else (s - 3, None)
            for i in range(4):
                top = post(base + i // 2, i % 2, valid, top, (i // 2) * seg)
                before[1, (1 + i) * G] = pltpu.bitcast(top[3], U32)
        else:
            job = jnp.where(s + 2 < n_seg, s // 2 + 1, 0) if u + 2 == _BLK else s // 2 + 1
            for i in range(live // 8):
                before[1, (1 + i) * G] = pltpu.bitcast(token_forms(job, i), U32)
        K(0); Q(0); V(0)
        for g in range(1, NG):
            K(g); Sc(g - 1); Q(g)
            if g > 1:
                PV(g - 2)
            V(g)
        order = [(c, n, j) for n in range(2) for c in (0, 1) for j in range(4)]
        order += [(c, n, j) for c in (2, 3) for n in range(2) for j in range(4)]
        for i, (c, n, j) in enumerate(order):
            if i == 5:
                Sc(NG - 1)
            if i == 9:
                PV(NG - 2)
            if i == 18:
                PV(NG - 1)
            O((c,), n, j)
        c1, c2 = [], []
        for n in range(2):
            r = [acc[n, j] for j in range(4)]
            o_tokens(odd, n, [x[n_mem:] for x in r])
            m = [x[:n_mem] for x in r]
            if odd:
                c1.append(m[0] + m[3])
                c2.append(m[1] + m[2])
            else:
                d = m[3] - m[0]
                c1.append(m[2] + d)
                c2.append(m[1] - d)
        return jnp.concatenate(c1 + c2, axis=1), top

    blk = _BLK * seg
    n_blk = n_seg // _BLK

    def out_copy(b):
        r = _rows(b * blk, blk)
        return pltpu.make_async_copy(ob.at[r], out_hbm.at[r], osem)

    def steps(b, carry):
        r0 = jnp.where(b + 1 < n_blk, b + 1, 0) * (_BLK * _PRE)
        units = [[(t, first, i)] for t, first in fill if not first for i in range(_BLK // 4)]
        units += [[(t, True, i), (t + 2, True, i)] for t, first in fill[_CH // 2::2] for i in range(_BLK // 4)]
        for u in range(_BLK):
            carry = step(b * _BLK + u, u, carry)
            if u + 1 < _BLK:
                for unit in units[len(units) * u // (_BLK - 1):len(units) * (u + 1) // (_BLK - 1)]:
                    for t, first, i in unit:
                        pre_tile(t, first, r0 + i * 32, 32)

        @pl.when(b == 0)
        def _():
            cxa[2].wait()

        @pl.when(b > 0)
        def _():
            out_copy(b - 1).start()

        @pl.when(b == 1)
        def _():
            for c in cf:
                c.start()
        return carry

    ninf = jnp.full((8, 128), -jnp.inf, F32)
    _, top = lax.fori_loop(0, n_blk, steps, (mem_ref[...].astype(F32), (ninf, sub, ninf, sub + 8)))
    for c in cf:
        c.wait()
    for n in range(2):
        o_tokens(0, n, [sum(_mm(osc[f, c, r0:r1], wo[f, c, :, n * 128:(n + 1) * 128]) for c in range(4))
                        for f, r0, r1, _ in o_plan[0]])
    for i in range(4):
        top = post(n_seg - 2 + i // 2, i % 2, None, top, (i // 2) * seg)
    b1, i1, b2, i2 = top
    out_copy(n_blk - 1).start()

    big = np.int32(1 << 30)
    m1 = jnp.max(b1, axis=0, keepdims=True)
    t1 = jnp.min(jnp.where(b1 == m1, i1, big), axis=0, keepdims=True)
    won = i1 == t1
    cb = jnp.where(won, b2, b1)
    ci = jnp.where(won, i2, i1)
    m2 = jnp.max(cb, axis=0, keepdims=True)
    t2 = jnp.min(jnp.where(cb == m2, ci, big), axis=0, keepdims=True)
    idx1 = jnp.clip(t1[0, 0], 0, S - 1)
    idx2 = jnp.clip(t2[0, 0], 0, S - 1)

    base1 = pl.multiple_of((idx1 // 16) * 16, 16)
    base2 = pl.multiple_of((idx2 // 16) * 16, 16)
    h = jnp.concatenate([hs[pl.ds(base1, 16), :], hs[pl.ds(base2, 16), :]], axis=0)
    hn = _layernorm(h)
    hb = hn.astype(BF16)
    gt = _rb(jnp.dot(hb, wg[...], preferred_element_type=F32))
    up = _rb(jnp.dot(hb, wu[...], preferred_element_type=F32))
    a = _rb(gt * _rb(jax.nn.sigmoid(gt))) * up
    y = _rb(jnp.dot(a.astype(BF16), wd[...], preferred_element_type=F32))
    rr = _rb(jnp.sum(hn * wr, axis=-1, keepdims=True))
    y = _rb(y * _rb(jax.nn.sigmoid(rr)))
    ri = lax.broadcasted_iota(jnp.int32, (32, D), 0)
    gi = jnp.where(ri < 16, ri + base1, ri + (base2 - 16))
    sel = (gi == idx1) | (gi == idx2)
    fix[...] = (h + _rb(hn + jnp.where(sel, y, 0.0))).astype(BF16)
    pltpu.make_async_copy(ob, out_hbm, osem).wait()
    f1 = pltpu.make_async_copy(fix.at[pl.ds(0, 16)], out_hbm.at[pl.ds(base1, 16)], sems.at[0])
    f2 = pltpu.make_async_copy(fix.at[pl.ds(16, 16)], out_hbm.at[pl.ds(base2, 16)], sems.at[12])
    f1.start()

    @pl.when(base1 != base2)
    def _():
        f2.start()
        f2.wait()
    f1.wait()


@functools.partial(jax.jit, static_argnames=("A_seg_len",))
def pallas_sequential_preLN__memory_aug_recurrent_mem_tr__moe_arch_mod__prompt_kernel(
    A_x, A_mem0, A_Wq, A_Wk, A_Wv, A_Wo, A_seg_len, B_x, B_w_r, B_w_gate, B_w_up, B_w_down,
):
    del B_x
    _, S, D = A_x.shape
    _, H, Dh = A_Wq.shape
    M = A_mem0.shape[1]
    F = B_w_gate.shape[1]
    seg = int(A_seg_len)
    n_seg = S // seg
    any_spec = pl.BlockSpec(memory_space=pl.ANY)
    vmem_spec = pl.BlockSpec(memory_space=pltpu.VMEM)
    out = pl.pallas_call(
        _kernel,
        out_shape=jax.ShapeDtypeStruct((S, D), A_x.dtype),
        in_specs=[any_spec] * 10,
        out_specs=any_spec,
        scratch_shapes=[
            pltpu.VMEM((M, D), BF16),
            pltpu.VMEM((D // 128, 128), BF16),
            pltpu.VMEM((n_seg, seg - _PRE, D), BF16),
            pltpu.VMEM((n_seg, _PRE, D), BF16),
            pltpu.VMEM((7, seg - _PRE, D // 2), F32),
            pltpu.VMEM((n_seg * _PRE // 2, D), U32),
            pltpu.VMEM((S, D), F32),
            pltpu.VMEM((2 * seg, D), F32),
            pltpu.VMEM((8, 128), U32),
            pltpu.VMEM((7, H // 8, seg, 4 * Dh), F32),
            pltpu.VMEM((3, H // 8, M, 4 * Dh), F32),
            pltpu.VMEM((H // 2, seg, Dh), F32),
            pltpu.VMEM((3 * H // _CH, D, _CH, Dh), BF16),
            pltpu.VMEM((3 * H, D // 2, Dh), U32),
            pltpu.VMEM((5, 3 * H // 2, D // 4, Dh), U32),
            pltpu.VMEM((3 * H, seg - _PRE, Dh), F32),
            pltpu.VMEM((3 * H, seg - _PRE, Dh), F32),
            pltpu.VMEM((3 * H // 2, 2 * _PRE, Dh), F32),
            pltpu.VMEM((3 * H, n_seg * _PRE, Dh), F32),
            pltpu.VMEM((H, Dh, D), BF16),
            pltpu.VMEM((7, H // 8, 2 * Dh, D // 2), U32),
            pltpu.VMEM((D, F), BF16),
            pltpu.VMEM((D, F), BF16),
            pltpu.VMEM((F, D), BF16),
            pltpu.VMEM((S, D), BF16),
            pltpu.VMEM((32, D), BF16),
            pltpu.SemaphoreType.DMA((25,)),
            pltpu.SemaphoreType.DMA,
        ],
        compiler_params=pltpu.CompilerParams(vmem_limit_bytes=110 * 1024 * 1024),
        name="rmt_mod",
    )(A_x.reshape(n_seg, seg, D), A_mem0.reshape(M, D), A_Wq, A_Wk, A_Wv, A_Wo,
      B_w_r.reshape(D // 128, 128), B_w_gate, B_w_up, B_w_down)
    return out.reshape(1, S, D)
```

```python
import functools

import jax
import jax.numpy as jnp
import numpy as np
from jax import lax
import jax.experimental.pallas as pl
import jax.experimental.pallas.tpu as pltpu

F32 = jnp.float32
BF16 = jnp.bfloat16
U32 = jnp.uint32

_NN = (((1,), (0,)), ((), ()))
_NT = (((1,), (1,)), ((), ()))
_PRE = 8
_BLK = 8
_CH = 16


def _rb(x):
    return x.astype(BF16).astype(F32)


def _layernorm(x):
    n = x.shape[-1]
    m = jnp.sum(x, axis=-1, keepdims=True) * (1.0 / n)
    xc = x - m
    v = jnp.sum(xc * xc, axis=-1, keepdims=True) * (1.0 / n)
    sd = _rb(jnp.sqrt(_rb(_rb(v) + 1e-5)))
    return _rb(_rb(x - _rb(m)) * (1.0 / sd))


def _mm(a, w_u32):
    return lax.dot_general(a, pltpu.bitcast(w_u32, BF16), _NN, preferred_element_type=F32)


def _forms(b11, b12, b21, b22):
    f11, f12, f21, f22 = (b.astype(F32) for b in (b11, b12, b21, b22))
    return ((f11 + f22).astype(BF16), b11, (f12 - f22).astype(BF16), (f21 - f11).astype(BF16), b22,
            (f11 + f12).astype(BF16), (f21 + f22).astype(BF16))


def _swap8(w):
    sub = lax.broadcasted_iota(jnp.int32, w[0].shape, 0)
    u = [pltpu.roll(w[-k % 8], -k % 8, 0) if k else w[0] for k in range(8)]
    for b in (1, 2, 4):
        u = [jnp.where((sub & b) != 0, u[(k - b) % 8], u[k]) for k in range(8)]
    return [pltpu.roll(u[j], -j % 8, 0) if j else u[0] for j in range(8)]


def _rows(start, size):
    return pl.ds(start, size) if isinstance(start, int) else pl.ds(pl.multiple_of(start, size), size)


def _kernel(x_hbm, mem_hbm, wq_hbm, wk_hbm, wv_hbm, wo_hbm, wr_hbm, wg_hbm, wu_hbm, wd_hbm,
            out_hbm,
            mem_ref, wr_ref, xa, xb, xn, xp, hs, att, zero, osc, osm, a12, raw, wqkv, wf, part, nxt, gam, pre, wo_raw, wo, wg, wu, wd, ob, fix, sems, osem):
    n_seg, seg, D = x_hbm.shape
    _, H, dh = wq_hbm.shape
    S = n_seg * seg
    n_mem = mem_ref.shape[0]
    live = seg - _PRE
    L = seg + n_mem
    G = 4
    NG = H // G
    scale = float(dh) ** -0.5
    w_hbm = (wk_hbm, wq_hbm, wv_hbm)
    NC = 3 * H // _CH

    def w_copy(c):
        return pltpu.make_async_copy(w_hbm[c // 2].at[:, pl.ds(_CH * (c % 2), _CH), :], raw.at[c], sems.at[c])

    NQ = 4
    dq = D // NQ
    c0 = [pltpu.make_async_copy(wk_hbm.at[pl.ds(i * dq, dq), pl.ds(0, _CH), :], raw.at[0, pl.ds(i * dq, dq)], sems.at[13 + i])
          for i in range(NQ)]
    cxb = pltpu.make_async_copy(x_hbm.at[:, pl.ds(live, _PRE), :], xb, sems.at[6])
    NB = NC - 2

    n_early = 2 * _BLK
    cxa = [pltpu.make_async_copy(x_hbm.at[r, pl.ds(0, live), :], xa.at[r], sems.at[17 + i])
           for i, r in enumerate((pl.ds(0, 2), pl.ds(2, n_early - 2), pl.ds(n_early, n_seg - n_early)))]

    def wo_copy(c):
        r = pl.ds(c * (H // NB), H // NB)
        return pltpu.make_async_copy(wo_hbm.at[r], wo_raw.at[r], sems.at[21 + c])

    cf = [pltpu.make_async_copy(a, b, sems.at[9 + i]) for i, (a, b) in enumerate(((wg_hbm, wg), (wu_hbm, wu), (wd_hbm, wd)))]

    cxb.start()
    cxa[0].start()
    for c in c0:
        c.start()
    for c in range(1, NC):
        w_copy(c).start()
    small = [pltpu.make_async_copy(mem_hbm, mem_ref, sems.at[7]), pltpu.make_async_copy(wr_hbm, wr_ref, sems.at[8])]
    for c in small:
        c.start()
    for c in range(NB):
        wo_copy(c).start()
    cxa[1].start()
    cxa[2].start()

    def relayout(c, i, after=(None, None)):
        a = pltpu.bitcast(raw[c, pl.ds(i * 16, 16)], U32).reshape(8, 2, _CH // 2, dh)
        ev, od = a[:, 0], a[:, 1]
        for b in range(2):
            e, o = (ev, od) if after[b] is None else (ev | after[b], od | after[b])
            if b == 0:
                w = (e & np.uint32(0xFFFF)) | (o << 16)
            else:
                w = (e >> 16) | (o & np.uint32(0xFFFF0000))
            t = _swap8([w[j] for j in range(8)])
            for j in range(_CH // 2):
                wqkv[c * _CH + 2 * j + b, _rows(i * 8, 8), :] = t[j]

    cxb.wait()
    cxa[0].wait()

    def ln_pre(i, _):
        v = xb[pl.ds(i * 32, 32)].astype(F32).reshape(32 * _PRE, D)
        xp[_rows(i * 128, 128), :] = pltpu.bitcast(_layernorm(v).astype(BF16), U32)
    lax.fori_loop(0, n_seg // 32, ln_pre, None)
    zero[...] = jnp.zeros(zero.shape, U32)

    for i in range(NQ):
        c0[i].wait()

        def rl0(t, _):
            relayout(0, 2 * t)
            relayout(0, 2 * t + 1)
        lax.fori_loop(i * dq // 32, (i + 1) * dq // 32, rl0, None)

    half = D // 2

    def pace(y, n):
        return [pltpu.bitcast(y[r:r + 8], U32) & zero[...] for r in (i * 60 // n * 8 for i in range(n))]

    def pre_tile(t, first, r0, r):
        k0 = half if first else 0
        y = _mm(pltpu.bitcast(xp[_rows(r0 // 2, r // 2), k0:], BF16), wqkv[t, k0 // 2:])
        pre[t, _rows(r0, r), :] = y
        return y

    def token_forms(job, j):
        r = pl.ds(j * 8, 8)
        top, bot = (_layernorm(xa[2 * job + i, r].astype(F32)) for i in range(2))
        a11, a12_, a21, a22 = top[:, :half], top[:, half:], bot[:, :half], bot[:, half:]
        fs = (a11 + a22, a21 + a22, a11, a22, a11 + a12_, a21 - a11, a12_ - a22)
        for f, v in enumerate(fs):
            xn[f, r, :] = v
        return fs[0][:, :128]

    def w_form(f, pair):
        if f == 1:
            return wqkv[2 * pair, :half // 2]
        if f == 4:
            return wqkv[2 * pair + 1, half // 2:]
        return wf[(0, None, 1, 2, None, 3, 4)[f], pair]

    def ahead_products(pair, lhs, early=False):
        order = [(j, f) for j in range(2) for f in (0, 5, 6)]
        at = 2 if early else 6
        m = {(j, f): _mm(lhs[f], w_form(f, pair + j)) for j, f in order[:at] + [(0, 1), (1, 1)] + order[at:]}
        for j in range(2):
            part[2 * (pair + j)] = (m[j, 0] + m[j, 6])[:live]
            part[2 * (pair + j) + 1] = (m[j, 0] + m[j, 5])[:live]
            gam[pair + j] = m[j, 1][:2 * _PRE]
        return m

    n_ahead = n_seg * _PRE
    n_pro = 3 * H - _CH
    fill = [(n_pro + 2 * j + 1, False) for j in range(_CH // 2)] + [(n_pro + 2 * j, True) for j in range(_CH // 2)]
    att[...] = jnp.zeros(att.shape, F32)
    for f in (0, 1, 5, 6):
        osc[f] = jnp.zeros(osc.shape[1:], F32)
    for j in range(live // 8):
        token_forms(0, j)
    for j in range(_CH // 2):
        pre_tile(2 * j, True, 0, n_ahead)

    def qkv_forms(pair, j, after):
        r = (pl.ds(j * 16, 16), pl.ds(half // 2 + j * 16, 16))
        w = [wqkv[2 * pair + b, r[a]] for a in range(2) for b in range(2)]
        if after is not None:
            w = [x | jnp.tile(after, (2, 1)) for x in w]
        fs = _forms(*(pltpu.bitcast(x, BF16) for x in w))
        for i, f in enumerate((0, 2, 3, 5, 6)):
            wf[i, pair, r[0]] = pltpu.bitcast(fs[f], U32)

    def pro_a(c, _):
        pltpu.make_async_copy(raw.at[c], raw.at[c], sems.at[c]).wait()
        for t in range(8):
            z = pace(pre_tile(c * _CH + (2 * t + 1 - _CH), False, 0, n_ahead), 16)
            for i in range(4):
                relayout(c, 4 * t + i, z[4 * i:4 * i + 2])
                qkv_forms(c * 8 + (t - 8), 2 * i, z[4 * i + 2])
                qkv_forms(c * 8 + (t - 8), 2 * i + 1, z[4 * i + 3])
    lax.fori_loop(1, NC, pro_a, None)
    for c in small:
        c.wait()

    def wo_forms(c, pair, j, after):
        def rows(head):
            w = pltpu.bitcast(wo_raw[c * 8 + 2 * pair + head, pl.ds(j * 16, 16), :], U32)
            w = pltpu.bitcast(w | jnp.tile(after, (1, D // 128)), BF16)
            return w[:, :D // 2], w[:, D // 2:]
        for f, w in enumerate(_forms(*rows(0), *rows(1))):
            wo[f, c, pl.ds(pair * (dh // 2) + j * 8, 8), :] = pltpu.bitcast(w, U32)

    def pro_b(c, _):
        wo_copy(c).wait()
        z = []
        for t in range(_CH // 2):
            y = pre_tile((c + 1) * _CH + 2 * t, True, 0, n_ahead)
            if t % 2:
                z += pace(y, 12)
        for i in range(16):
            qkv_forms(n_pro // 2 + c * 2 + i // 8, i % 8, z[i])
        for i in range(32):
            wo_forms(c, i // 8, i % 8, z[16 + i])
        lhs = {f: xn[f].astype(BF16) for f in (0, 5, 6)}
        lhs[1] = pltpu.bitcast(xp[0:_PRE, :half], BF16)
        for i in range(NC):
            ahead_products(c * 2 + i * 8, lhs)
        for i in range(4):
            pre_tile(n_pro + c * 4 + (1, 3, 0, 2)[i], i > 1, 0, _BLK * _PRE)
    lax.fori_loop(0, NB, pro_b, None)
    cxa[1].wait()

    def pos(i):
        return jnp.where(i < live, i + n_mem, jnp.where(i < live + n_mem, i - live, i))
    row = pos(lax.broadcasted_iota(jnp.int32, (L, L), 0))
    col = pos(lax.broadcasted_iota(jnp.int32, (L, L), 1))
    mask = (row < n_mem) | (row >= col)
    c_exp = scale * float(np.log2(np.e))
    neg = -1e9 / scale

    wr = wr_ref[...].astype(F32)
    wr = jnp.concatenate([wr[i:i + 1, :] for i in range(D // 128)], axis=1)
    sub = lax.broadcasted_iota(jnp.int32, (8, 128), 0)

    def post(s, part_, valid, top, at):
        b1, i1, b2, i2 = top
        r = _rows(s * seg + part_ * 16, 16)
        if part_ == 0:
            x = xa[s, 0:16].astype(F32)
        else:
            x = jnp.concatenate([xa[s, 16:live].astype(F32), xb[s].astype(F32)], axis=0)
        h = _rb(x + _rb(att[at + part_ * 16:at + part_ * 16 + 16]))
        hs[r, :] = h
        hn = _layernorm(h)
        ob[r, :] = (h + hn).astype(BF16)
        rr = _rb(jnp.sum(hn * wr, axis=-1, keepdims=True))
        for j in range(2):
            val = jnp.broadcast_to(rr[8 * j:8 * j + 8], (8, 128))
            if valid is not None:
                val = jnp.where(valid, val, -jnp.inf)
            idx = sub + (s * seg + part_ * 16 + 8 * j)
            g1 = val > b1
            g2 = val > b2
            b2 = jnp.where(g1, b1, jnp.where(g2, val, b2))
            i2 = jnp.where(g1, i1, jnp.where(g2, idx, i2))
            b1 = jnp.where(g1, val, b1)
            i1 = jnp.where(g1, idx, i1)
        return b1, i1, b2, i2

    o_plan = (((0, 0, seg, 1), (5, 0, seg, 0), (6, 0, seg, 1), (1, seg // 2, seg, 2)),
              ((3, 0, seg, 1), (2, 0, seg, 0), (4, 0, seg, 2), (1, 0, seg // 2, 2)))

    def o_tokens(odd, n, r):
        lo, hi = pl.ds(n * 128, 128), pl.ds(D // 2 + n * 128, 128)
        hs_ = seg // 2
        if odd:
            m4, m3, m5, m2 = r
            att[0:seg, lo] = m4 - m5
            att[0:seg, hi] = m3 + m5
            att[seg:seg + hs_, lo] = m4[:hs_] + m2
            att[seg + hs_:2 * seg, lo] = m4[hs_:]
            att[seg:seg + hs_, hi] = m3[:hs_] - m2
            att[seg + hs_:2 * seg, hi] = m3[hs_:]
        else:
            m1, m6, m7, m2 = r
            att[0:seg, lo] += m1 + m7
            att[seg + hs_:2 * seg, lo] += m2
            t = m1 + m6
            att[seg:seg + hs_, hi] += t[:hs_]
            att[seg + hs_:2 * seg, hi] += t[hs_:] - m2

    def step(s, u, carry):
        odd = u % 2
        mem, top = carry
        a1, a2 = mem[:, :half], mem[:, half:]
        a3 = a1 + a2
        if odd:
            job = jnp.where(s + 1 < n_seg, (s + 1) // 2, 0) if u + 1 == _BLK else (s + 1) // 2
            lhs = {f: jnp.concatenate([xn[f], a], axis=0).astype(BF16) for f, a in ((0, a2), (5, a1), (6, a2))}
            lhs[1] = jnp.concatenate([pltpu.bitcast(xp[_rows(job * _PRE, _PRE), :half], BF16).astype(F32), a3], axis=0)
        else:
            lhs = {f: jnp.concatenate([xn[f], a], axis=0).astype(BF16) for f, a in ((1, a3), (2, a1), (3, a2), (4, a3))}
        pr = _rows(s * _PRE, _PRE)
        k, q, v, p = {}, {}, {}, {}
        before = {}
        acc = {}

        def proj(dst, m, g):
            t0 = m * H + g * G
            ahead = [pre[t, pr, :] for t in range(t0, t0 + G)]
            for j in range(0, G, 2):
                ahead[j] = ahead[j] + gam[(t0 + j) // 2, pl.ds(odd * _PRE, _PRE)]
            if (m, g) in before:
                ahead[1] = pltpu.bitcast(pltpu.bitcast(ahead[1], U32) | (before[m, g] & zero[...]), F32)
            if odd:
                y = ahead_products(t0 // 2, lhs, m == 2)
            for j in range(0, G, 2):
                t, i = t0 + j, g * G + j
                if odd:
                    m1, m6, m7, mg = (y[j // 2, f] for f in (0, 5, 6, 1))
                    d = mg[2 * _PRE:] - m1[live:]
                    dst[i] = jnp.concatenate([nxt[t], m7[live:] + d, ahead[j]], axis=0)
                    dst[i + 1] = jnp.concatenate([nxt[t + 1], m6[live:] - d, ahead[j + 1]], axis=0)
                else:
                    m2, m4, m3, m5 = (_mm(lhs[f], w_form(f, t // 2)) for f in (1, 3, 2, 4))
                    y = m2 + m4
                    nxt[t] = y[:live]
                    nxt[t + 1] = part[t + 1] + (m3 - m2)[:live]
                    dst[i] = jnp.concatenate([part[t] + (m4 - m5)[:live], y[live:], ahead[j]], axis=0)
                    dst[i + 1] = jnp.concatenate([m3 + m5, ahead[j + 1]], axis=0)

        def K(g):
            proj(k, 0, g)

        def Q(g):
            proj(q, 1, g)

        def V(g):
            proj(v, 2, g)

        def Sc(g):
            for i in range(g * G, (g + 1) * G):
                sc = lax.dot_general(q[i], k[i].astype(BF16), _NT, preferred_element_type=F32)
                sc = jnp.where(mask, sc, neg)
                e = jnp.exp2((sc - jnp.max(sc, axis=-1, keepdims=True)) * c_exp)
                l = jnp.sum(e, axis=-1, keepdims=True)
                r = pl.reciprocal(l, approx=True)
                p[i] = e * (r * (2.0 - l * r))

        def PV(g):
            o = [lax.dot_general(p[i], v[i].astype(BF16), _NN, preferred_element_type=F32)
                 for i in range(g * G, (g + 1) * G)]
            for j in range(G // 2):
                t = g * (G // 2) + j
                c, cs = t // 4, pl.ds((t % 4) * dh, dh)
                m1, m2 = (x[live:live + n_mem] for x in o[2 * j:2 * j + 2])
                osm[0, c, :, cs] = m1
                osm[1, c, :, cs] = m2
                osm[2, c, :, cs] = m1 + m2
                x1, x2 = (jnp.concatenate([x[:live], x[live + n_mem:]], axis=0) for x in o[2 * j:2 * j + 2])
                if odd:
                    y1, y2 = osc[2, c, :, cs], a12[t]
                    osc[3, c, :, cs] = x2
                    osc[1, c, :, cs] = x1 + x2
                    osc[0, c, :, cs] = y1 + x2
                    osc[5, c, :, cs] = x1 - y1
                    osc[6, c, :, cs] = y2 - x2
                else:
                    osc[2, c, :, cs] = x1
                    osc[4, c, :, cs] = x1 + x2
                    a12[t] = x2

        def O(cs_, n, j):
            f, r0, r1, fm = o_plan[odd][j]
            t = acc.get((n, j))
            for c in cs_:
                lhs = jnp.concatenate([osm[fm, c], osc[f, c, r0:r1]], axis=0)
                y = _mm(lhs, wo[f, c, :, n * 128:(n + 1) * 128])
                t = y if t is None else t + y
            acc[n, j] = t

        if odd:
            base, valid = (jnp.maximum(s - 3, 0), s > 1) if u == 1 else (s - 3, None)
            for i in range(4):
                top = post(base + i // 2, i % 2, valid, top, (i // 2) * seg)
                before[1, 1 + i] = pltpu.bitcast(top[3], U32)
        else:
            job = jnp.where(s + 2 < n_seg, s // 2 + 1, 0) if u + 2 == _BLK else s // 2 + 1
            for i in range(live // 8):
                before[1, 1 + i] = pltpu.bitcast(token_forms(job, i), U32)
        K(0); Q(0); V(0)
        for g in range(1, NG):
            K(g); Sc(g - 1); Q(g)
            if g > 1:
                PV(g - 2)
            V(g)
        order = [(c, n, j) for n in range(2) for c in (0, 1) for j in range(4)]
        order += [(c, n, j) for c in (2, 3) for n in range(2) for j in range(4)]
        for i, (c, n, j) in enumerate(order):
            if i == 5:
                Sc(NG - 1)
            if i == 9:
                PV(NG - 2)
            if i == 18:
                PV(NG - 1)
            O((c,), n, j)
        c1, c2 = [], []
        for n in range(2):
            r = [acc[n, j] for j in range(4)]
            o_tokens(odd, n, [x[n_mem:] for x in r])
            m = [x[:n_mem] for x in r]
            if odd:
                c1.append(m[0] + m[3])
                c2.append(m[1] + m[2])
            else:
                d = m[3] - m[0]
                c1.append(m[2] + d)
                c2.append(m[1] - d)
        return jnp.concatenate(c1 + c2, axis=1), top

    blk = _BLK * seg
    n_blk = n_seg // _BLK

    def out_copy(b):
        r = _rows(b * blk, blk)
        return pltpu.make_async_copy(ob.at[r], out_hbm.at[r], osem)

    def steps(b, carry):
        r0 = jnp.where(b + 1 < n_blk, b + 1, 0) * (_BLK * _PRE)
        units = [[(t, first, i)] for t, first in fill if not first for i in range(_BLK // 4)]
        units += [[(t, True, i), (t + 2, True, i)] for t, first in fill[_CH // 2::2] for i in range(_BLK // 4)]
        for u in range(_BLK):
            carry = step(b * _BLK + u, u, carry)
            if u + 1 < _BLK:
                for unit in units[len(units) * u // (_BLK - 1):len(units) * (u + 1) // (_BLK - 1)]:
                    for t, first, i in unit:
                        pre_tile(t, first, r0 + i * 32, 32)

        @pl.when(b == 0)
        def _():
            cxa[2].wait()

        @pl.when(b > 0)
        def _():
            out_copy(b - 1).start()

        @pl.when(b == 1)
        def _():
            for c in cf:
                c.start()
        return carry

    ninf = jnp.full((8, 128), -jnp.inf, F32)
    _, top = lax.fori_loop(0, n_blk, steps, (mem_ref[...].astype(F32), (ninf, sub, ninf, sub + 8)))
    for c in cf:
        c.wait()
    for n in range(2):
        o_tokens(0, n, [sum(_mm(osc[f, c, r0:r1], wo[f, c, :, n * 128:(n + 1) * 128]) for c in range(4))
                        for f, r0, r1, _ in o_plan[0]])
    for i in range(4):
        top = post(n_seg - 2 + i // 2, i % 2, None, top, (i // 2) * seg)
    b1, i1, b2, i2 = top
    out_copy(n_blk - 1).start()

    big = np.int32(1 << 30)
    m1 = jnp.max(b1, axis=0, keepdims=True)
    t1 = jnp.min(jnp.where(b1 == m1, i1, big), axis=0, keepdims=True)
    won = i1 == t1
    cb = jnp.where(won, b2, b1)
    ci = jnp.where(won, i2, i1)
    m2 = jnp.max(cb, axis=0, keepdims=True)
    t2 = jnp.min(jnp.where(cb == m2, ci, big), axis=0, keepdims=True)
    idx1 = jnp.clip(t1[0, 0], 0, S - 1)
    idx2 = jnp.clip(t2[0, 0], 0, S - 1)

    base1 = pl.multiple_of((idx1 // 16) * 16, 16)
    base2 = pl.multiple_of((idx2 // 16) * 16, 16)
    h = jnp.concatenate([hs[pl.ds(base1, 16), :], hs[pl.ds(base2, 16), :]], axis=0)
    hn = _layernorm(h)
    hb = hn.astype(BF16)
    gt = _rb(jnp.dot(hb, wg[...], preferred_element_type=F32))
    up = _rb(jnp.dot(hb, wu[...], preferred_element_type=F32))
    a = _rb(gt * _rb(jax.nn.sigmoid(gt))) * up
    y = _rb(jnp.dot(a.astype(BF16), wd[...], preferred_element_type=F32))
    rr = _rb(jnp.sum(hn * wr, axis=-1, keepdims=True))
    y = _rb(y * _rb(jax.nn.sigmoid(rr)))
    ri = lax.broadcasted_iota(jnp.int32, (32, D), 0)
    gi = jnp.where(ri < 16, ri + base1, ri + (base2 - 16))
    sel = (gi == idx1) | (gi == idx2)
    fix[...] = (h + _rb(hn + jnp.where(sel, y, 0.0))).astype(BF16)
    pltpu.make_async_copy(ob, out_hbm, osem).wait()
    f1 = pltpu.make_async_copy(fix.at[pl.ds(0, 16)], out_hbm.at[pl.ds(base1, 16)], sems.at[0])
    f2 = pltpu.make_async_copy(fix.at[pl.ds(16, 16)], out_hbm.at[pl.ds(base2, 16)], sems.at[12])
    f1.start()

    @pl.when(base1 != base2)
    def _():
        f2.start()
        f2.wait()
    f1.wait()


@functools.partial(jax.jit, static_argnames=("A_seg_len",))
def pallas_sequential_preLN__memory_aug_recurrent_mem_tr__moe_arch_mod__prompt_kernel(
    A_x, A_mem0, A_Wq, A_Wk, A_Wv, A_Wo, A_seg_len, B_x, B_w_r, B_w_gate, B_w_up, B_w_down,
):
    del B_x
    _, S, D = A_x.shape
    _, H, Dh = A_Wq.shape
    M = A_mem0.shape[1]
    F = B_w_gate.shape[1]
    seg = int(A_seg_len)
    n_seg = S // seg
    any_spec = pl.BlockSpec(memory_space=pl.ANY)
    vmem_spec = pl.BlockSpec(memory_space=pltpu.VMEM)
    out = pl.pallas_call(
        _kernel,
        out_shape=jax.ShapeDtypeStruct((S, D), A_x.dtype),
        in_specs=[any_spec] * 10,
        out_specs=any_spec,
        scratch_shapes=[
            pltpu.VMEM((M, D), BF16),
            pltpu.VMEM((D // 128, 128), BF16),
            pltpu.VMEM((n_seg, seg - _PRE, D), BF16),
            pltpu.VMEM((n_seg, _PRE, D), BF16),
            pltpu.VMEM((7, seg - _PRE, D // 2), F32),
            pltpu.VMEM((n_seg * _PRE // 2, D), U32),
            pltpu.VMEM((S, D), F32),
            pltpu.VMEM((2 * seg, D), F32),
            pltpu.VMEM((8, 128), U32),
            pltpu.VMEM((7, H // 8, seg, 4 * Dh), F32),
            pltpu.VMEM((3, H // 8, M, 4 * Dh), F32),
            pltpu.VMEM((H // 2, seg, Dh), F32),
            pltpu.VMEM((3 * H // _CH, D, _CH, Dh), BF16),
            pltpu.VMEM((3 * H, D // 2, Dh), U32),
            pltpu.VMEM((5, 3 * H // 2, D // 4, Dh), U32),
            pltpu.VMEM((3 * H, seg - _PRE, Dh), F32),
            pltpu.VMEM((3 * H, seg - _PRE, Dh), F32),
            pltpu.VMEM((3 * H // 2, 2 * _PRE, Dh), F32),
            pltpu.VMEM((3 * H, n_seg * _PRE, Dh), F32),
            pltpu.VMEM((H, Dh, D), BF16),
            pltpu.VMEM((7, H // 8, 2 * Dh, D // 2), U32),
            pltpu.VMEM((D, F), BF16),
            pltpu.VMEM((D, F), BF16),
            pltpu.VMEM((F, D), BF16),
            pltpu.VMEM((S, D), BF16),
            pltpu.VMEM((32, D), BF16),
            pltpu.SemaphoreType.DMA((25,)),
            pltpu.SemaphoreType.DMA,
        ],
        compiler_params=pltpu.CompilerParams(vmem_limit_bytes=110 * 1024 * 1024),
        name="rmt_mod",
    )(A_x.reshape(n_seg, seg, D), A_mem0.reshape(M, D), A_Wq, A_Wk, A_Wv, A_Wo,
      B_w_r.reshape(D // 128, 128), B_w_gate, B_w_up, B_w_down)
    return out.reshape(1, S, D)
```

```python
import functools

import jax
import jax.numpy as jnp
import numpy as np
from jax import lax
import jax.experimental.pallas as pl
import jax.experimental.pallas.tpu as pltpu

F32 = jnp.float32
BF16 = jnp.bfloat16
U32 = jnp.uint32

_NN = (((1,), (0,)), ((), ()))
_NT = (((1,), (1,)), ((), ()))
_PRE = 8
_BLK = 8
_CH = 8
_G = 4
M1, M2, M3, M4, M5, M6, M7 = range(7)


def _rb(x):
    return x.astype(BF16).astype(F32)


def _layernorm(x):
    n = x.shape[-1]
    m = jnp.sum(x, axis=-1, keepdims=True) * (1.0 / n)
    xc = x - m
    v = jnp.sum(xc * xc, axis=-1, keepdims=True) * (1.0 / n)
    sd = _rb(jnp.sqrt(_rb(_rb(v) + 1e-5)))
    return _rb(_rb(x - _rb(m)) * (1.0 / sd))


def _mm(a, w):
    return lax.dot_general(a, pltpu.bitcast(w, BF16), _NN, preferred_element_type=F32)


def _left_forms(a11, a12, a21, a22):
    return a11 + a22, a21 + a22, a11, a22, a11 + a12, a21 - a11, a12 - a22


def _right_forms(b11, b12, b21, b22):
    f11, f12, f21, f22 = (pltpu.bitcast(b, BF16).astype(F32) for b in (b11, b12, b21, b22))

    def pack(x):
        return pltpu.bitcast(x.astype(BF16), U32)
    return pack(f11 + f22), b11, pack(f12 - f22), pack(f21 - f11), b22, pack(f11 + f12), pack(f21 + f22)


def _swap8(w):
    sub = lax.broadcasted_iota(jnp.int32, w[0].shape, 0)
    u = [pltpu.roll(w[-k % 8], -k % 8, 0) if k else w[0] for k in range(8)]
    for b in (1, 2, 4):
        u = [jnp.where((sub & b) != 0, u[(k - b) % 8], u[k]) for k in range(8)]
    return [pltpu.roll(u[j], -j % 8, 0) if j else u[0] for j in range(8)]


def _rows(start, size):
    return pl.ds(start, size) if isinstance(start, int) else pl.ds(pl.multiple_of(start, size), size)


def _kernel(x_hbm, mem_hbm, wq_hbm, wk_hbm, wv_hbm, wo_hbm, wr_hbm, wg_hbm, wu_hbm, wd_hbm,
            out_hbm,
            mem_ref, wr_ref, xa, xb, xl, xp, xg, raw, wp, pre, part, nxt, wo_raw, wo, ol, om, o12, att, hs,
            wg, wu, wd, ob, fix, zero, sem, out_sem):
    n_seg, seg, D = x_hbm.shape
    _, H, dh = wq_hbm.shape
    S = n_seg * seg
    n_job = n_seg // 2
    n_mem = mem_ref.shape[0]
    live = seg - _PRE
    half = D // 2
    NG = H // _G
    NC = 3 * H // _CH

    def w_copies(c):
        w = (wk_hbm, wq_hbm, wv_hbm)[c * _CH // H]
        return [pltpu.make_async_copy(w.at[pl.ds(i * half, half), pl.ds(c * _CH % H, _CH), :],
                                      raw.at[c, :, pl.ds(i * _CH, _CH), :], sem.at[11 + c]) for i in range(2)]

    def w_wait(c):
        pltpu.make_async_copy(raw.at[c], raw.at[c], sem.at[11 + c]).wait()

    def wo_copy(g):
        r = pl.ds(g * _G, _G)
        return pltpu.make_async_copy(wo_hbm.at[r], wo_raw.at[r], sem.at[11 + NC + g])

    def xa_copy(i, lo, hi):
        r = pl.ds(lo, hi - lo)
        return pltpu.make_async_copy(x_hbm.at[r, pl.ds(0, live), :], xa.at[r], sem.at[i])

    first = [pltpu.make_async_copy(x_hbm.at[:, pl.ds(live, _PRE), :], xb, sem.at[0]), xa_copy(1, 0, 2)]
    second = [pltpu.make_async_copy(mem_hbm, mem_ref, sem.at[2]), pltpu.make_async_copy(wr_hbm, wr_ref, sem.at[3]),
              xa_copy(4, 2, 2 * _BLK)]
    third = xa_copy(5, 2 * _BLK, n_seg)
    ffn = [pltpu.make_async_copy(a, b, sem.at[6 + i])
           for i, (a, b) in enumerate(((wg_hbm, wg), (wu_hbm, wu), (wd_hbm, wd)))]
    wo_from = NC - 1 - NG
    for cp in first:
        cp.start()
    for c in range(NC):
        for cp in w_copies(c):
            cp.start()
        if wo_from <= c < wo_from + NG:
            wo_copy(c - wo_from).start()
    for cp in second + [third]:
        cp.start()

    def pace(y):
        return pltpu.bitcast(y, U32) & zero[...]

    def prepare_qkv(c, i, after):
        a = pltpu.bitcast(raw[c, pl.ds(i * 16, 16)], U32).reshape(8, 2, _CH, dh)
        t = []
        for b in range(2):
            e, o = (a[:, k] if after is None else a[:, k] | after[b] for k in range(2))
            w = (e >> 16) | (o & np.uint32(0xFFFF0000)) if b else (e & np.uint32(0xFFFF)) | (o << 16)
            t.append(_swap8([w[j] for j in range(8)]))
        n = _CH // 2
        for j in range(n):
            blocks = [t[0][j], t[1][j], t[0][n + j], t[1][n + j]]
            if after is not None:
                blocks = [x | after[2 + j // 2] for x in blocks]
            for f, w in enumerate(_right_forms(*blocks)):
                wp[c * n + j, f, _rows(i * 8, 8), :] = w

    def prepare_wo(g, i, after):
        pair, j = i // 8, i % 8
        top, bot = (pltpu.bitcast(wo_raw[g * _G + 2 * pair + b, pl.ds(j * 16, 16), :], U32)
                    | jnp.tile(after, (1, D // 128)) for b in range(2))
        forms = _right_forms(top[:, :half], top[:, half:], bot[:, :half], bot[:, half:])
        for f, w in enumerate(forms):
            wo[f, _rows(g * dh + i * 8, 8), :] = w

    def live_forms(job, j):
        r = pl.ds(j * 8, 8)
        top, bot = (_layernorm(xa[2 * job + b, r].astype(F32)) for b in range(2))
        forms = _left_forms(top[:, :half], top[:, half:], bot[:, :half], bot[:, half:])
        for f, v in enumerate(forms):
            xl[f, r, :] = v
        return forms[M1][:, :128]

    def ahead(pair, n_pair, job, n, start=False):
        r = n * _PRE

        def product(j, f):
            lhs = pltpu.bitcast(xp[f, _rows(job * (_PRE // 2), r // 2), :], BF16)
            if start and f in (M1, M6, M7):
                lhs = jnp.concatenate([lhs, xl[f].astype(BF16)], axis=0)
            return _mm(lhs, wp[pair + j, f])
        if n_pair == 1:
            order = [(0, f) for f in (M1, M6, M7, M4, M3, M5)]
        else:
            order = [(0, M1), (0, M6), (0, M7), (1, M7), (0, M4), (1, M4), (0, M3), (0, M5),
                     (1, M1), (1, M6), (1, M3), (1, M5)]
        m = {jf: product(*jf) for jf in order}
        rows = _rows(job * _PRE, r)
        for j in range(n_pair):
            t = 2 * (pair + j)
            c11, c22 = m[j, M1] + m[j, M7], m[j, M1] + m[j, M6]
            if start:
                part[t] = c11[r:]
                part[t + 1] = c22[r:]
            pre[t, 0, rows, :] = c11[:r] + m[j, M4] - m[j, M5]
            pre[t + 1, 0, rows, :] = m[j, M3] + m[j, M5]
            pre[t, 1, rows, :] = m[j, M4]
            pre[t + 1, 1, rows, :] = c22[:r] + m[j, M3]
        return [m[jf] for jf in order[::2]]

    zero[...] = jnp.zeros(zero.shape, U32)
    att[...] = jnp.zeros(att.shape, F32)
    for f in (M1, M2, M6, M7):
        ol[f] = jnp.zeros(ol.shape[1:], F32)
    for cp in first:
        cp.wait()

    def pre_forms(i, _):
        n = n_job // 2
        v = _layernorm(xb[pl.ds(i * 2 * n, 2 * n)].astype(F32).reshape(2 * n * _PRE, D)).reshape(n, 2, _PRE, D)
        top, bot = (v[:, b].reshape(n * _PRE, D) for b in range(2))
        for f, u in enumerate(_left_forms(top[:, :half], top[:, half:], bot[:, :half], bot[:, half:])):
            if f == M2:
                xg[_rows(i * n * _PRE, n * _PRE), :] = u
            else:
                xp[f, _rows(i * n * _PRE // 2, n * _PRE // 2), :] = pltpu.bitcast(u.astype(BF16), U32)
    lax.fori_loop(0, 2, pre_forms, None)
    for j in range(live // 8):
        live_forms(0, j)

    w_wait(0)
    lax.fori_loop(0, half // 16, lambda i, _: prepare_qkv(0, i, None), None)

    def prologue(with_wo, c, _):
        w_wait(c)
        if with_wo:
            wo_copy(c - wo_from).wait()
        z = [pace(y[r:r + 8]) for j in (0, 2) for y in ahead(c * (_CH // 2) + (j - _CH // 2), 2, 0, n_job, True)
             for r in range(0, 256, 40)]
        for i in range(half // 16):
            prepare_qkv(c, i, z[5 * i:5 * i + 4])
            if with_wo:
                prepare_wo(c - wo_from, i, z[5 * i + 4])
    lax.fori_loop(1, wo_from, functools.partial(prologue, False), None)
    lax.fori_loop(wo_from, NC - 1, functools.partial(prologue, True), None)

    kept = (NC - 2) * (_CH // 2)
    w_wait(NC - 1)
    for cp in second:
        cp.wait()
    for i in range(half // 16):
        prepare_qkv(NC - 1, i, None)
    for pair in range(kept, 3 * H // 2, 2):
        ahead(pair, 2, 0, _BLK // 2, True)

    def pos(i):
        return jnp.where(i < live, i + n_mem, jnp.where(i < live + n_mem, i - live, i))
    row = pos(lax.broadcasted_iota(jnp.int32, (seg + n_mem, seg + n_mem), 0))
    col = pos(lax.broadcasted_iota(jnp.int32, (seg + n_mem, seg + n_mem), 1))
    mask = (row < n_mem) | (row >= col)
    scale = float(dh) ** -0.5

    wr = wr_ref[...].astype(F32)
    wr = jnp.concatenate([wr[i:i + 1, :] for i in range(D // 128)], axis=1)
    sub = lax.broadcasted_iota(jnp.int32, (8, 128), 0)

    def finish(s0, i, valid, top):
        b1, i1, b2, i2 = top
        s = s0 + i // 2
        if i % 2 == 0:
            x = xa[s, 0:16].astype(F32)
        else:
            x = jnp.concatenate([xa[s, 16:live].astype(F32), xb[s].astype(F32)], axis=0)
        r = _rows(s0 * seg + i * 16, 16)
        h = _rb(x + _rb(att[i * 16:i * 16 + 16]))
        hn = _layernorm(h)
        hs[0, r, :] = h
        hs[1, r, :] = hn
        ob[r, :] = (h + hn).astype(BF16)
        score = _rb(jnp.sum(hn * wr, axis=-1, keepdims=True))
        for j in range(2):
            val = jnp.broadcast_to(score[8 * j:8 * j + 8], (8, 128))
            if valid is not None:
                val = jnp.where(valid, val, -jnp.inf)
            idx = sub + (s0 * seg + i * 16 + 8 * j)
            g1 = val > b1
            g2 = val > b2
            b2 = jnp.where(g1, b1, jnp.where(g2, val, b2))
            i2 = jnp.where(g1, i1, jnp.where(g2, idx, i2))
            b1 = jnp.where(g1, val, b1)
            i1 = jnp.where(g1, idx, i1)
        return b1, i1, b2, i2

    mem_operand = {M1: 1, M2: 2, M3: 0, M4: 1, M5: 2, M6: 0, M7: 1}

    def mem_result(m):
        if M3 in m:
            return m[M2] + m[M4], m[M3] + m[M5]
        d = m[M2] - m[M1]
        return m[M7] + d, m[M6] - d

    hseg = seg // 2
    out_plan = (((M1, 0, seg), (M6, 0, seg), (M2, hseg, seg), (M7, 0, seg)),
                ((M4, 0, seg), (M3, 0, seg), (M2, 0, hseg), (M5, 0, seg)))

    def out_product(f, r0, r1, c, n, with_mem=True):
        lhs = ol[f, c, r0:r1]
        if with_mem:
            lhs = jnp.concatenate([om[mem_operand[f], c], lhs], axis=0)
        return _mm(lhs, wo[f, c * 2 * dh:(c + 1) * 2 * dh, n * 128:(n + 1) * 128])

    def out_tokens(n, m):
        lo, hi = pl.ds(n * 128, 128), pl.ds(half + n * 128, 128)
        if M3 in m:
            att[0:seg, lo] = m[M4] - m[M5]
            att[0:seg, hi] = m[M3] + m[M5]
            att[seg:seg + hseg, lo] = m[M4][:hseg] + m[M2]
            att[seg + hseg:2 * seg, lo] = m[M4][hseg:]
            att[seg:seg + hseg, hi] = m[M3][:hseg] - m[M2]
            att[seg + hseg:2 * seg, hi] = m[M3][hseg:]
        else:
            att[0:seg, lo] += m[M1] + m[M7]
            att[seg + hseg:2 * seg, lo] += m[M2]
            t = m[M1] + m[M6]
            att[seg:seg + hseg, hi] += t[:hseg]
            att[seg + hseg:2 * seg, hi] += t[hseg:] - m[M2]

    def step(b, u, carry):
        mem, top = carry
        odd = u % 2
        job = b * (_BLK // 2) + u // 2
        pr = _rows(job * _PRE, _PRE)
        a = (mem[:, :half], mem[:, half:], mem[:, :half] + mem[:, half:])
        lhs = {f: jnp.concatenate([xg[pr, :] if odd and f == M2 else xl[f], a[mem_operand[f]]], axis=0).astype(BF16)
               for f in ((M1, M6, M7, M2) if odd else (M2, M3, M4, M5))}
        needs = {}
        if odd:
            s0, valid = (jnp.maximum(2 * job - 2, 0), b > 0) if u == 1 else (2 * job - 2, None)
            for i in range(4):
                top = finish(s0, i, valid, top)
                needs[1, 1 + i] = top[3]
        else:
            nj = jnp.where(job + 1 < n_job, job + 1, 0) if u + 2 == _BLK else job + 1
            for i in range(live // 8):
                needs[1, 1 + i] = live_forms(nj, i)
        kqv, p, acc = ({}, {}, {}), {}, {}

        def project(w, g):
            t0 = w * H + g * _G
            early = [pre[t, odd, pr, :] for t in range(t0, t0 + _G)]
            if (w, g) in needs:
                early[0] = pltpu.bitcast(pltpu.bitcast(early[0], U32) | pace(needs[w, g]), F32)
            if odd:
                order = [(j, f) for j in range(2) for f in (M1, M6, M7)]
                at = 2 if w == 2 else 6
                order = order[:at] + [(0, M2), (1, M2)] + order[at:]
            else:
                order = [(j, f) for j in range(2) for f in (M2, M4, M3, M5)]
            y = {(j, f): _mm(lhs[f], wp[t0 // 2 + j, f]) for j, f in order}
            for j in range(2):
                t = t0 + 2 * j
                m = {f: y[j, f][:-n_mem] for f in lhs}
                c1, c2 = mem_result({f: y[j, f][-n_mem:] for f in lhs})
                if odd:
                    rows = ((nxt[t], c1, early[2 * j] + m[M2]), (nxt[t + 1], c2, early[2 * j + 1] - m[M2]))
                    part[t] = m[M1] + m[M7]
                    part[t + 1] = m[M1] + m[M6]
                else:
                    rows = ((part[t] + (m[M4] - m[M5]), c1, early[2 * j]), (m[M3] + m[M5], c2, early[2 * j + 1]))
                    nxt[t] = m[M2] + m[M4]
                    nxt[t + 1] = part[t + 1] + (m[M3] - m[M2])
                for i in range(2):
                    kqv[w][g * _G + 2 * j + i] = jnp.concatenate(rows[i], axis=0)

        def scores(g):
            for i in range(g * _G, (g + 1) * _G):
                sc = lax.dot_general(kqv[1][i], kqv[0][i].astype(BF16), _NT, preferred_element_type=F32)
                sc = jnp.where(mask, sc, -1e9 / scale)
                e = jnp.exp2((sc - jnp.max(sc, axis=-1, keepdims=True)) * (scale * float(np.log2(np.e))))
                l = jnp.sum(e, axis=-1, keepdims=True)
                r = pl.reciprocal(l, approx=True)
                p[i] = e * (r * (2.0 - l * r))

        def values(g):
            o = [lax.dot_general(p[i], kqv[2][i].astype(BF16), _NN, preferred_element_type=F32)
                 for i in range(g * _G, (g + 1) * _G)]
            for j in range(2):
                t = 2 * g + j
                c, cs = t // 4, pl.ds((t % 4) * dh, dh)
                m1, m2 = (x[live:live + n_mem] for x in o[2 * j:2 * j + 2])
                om[0, c, :, cs] = m1
                om[1, c, :, cs] = m2
                om[2, c, :, cs] = m1 + m2
                x1, x2 = (jnp.concatenate([x[:live], x[live + n_mem:]], axis=0) for x in o[2 * j:2 * j + 2])
                if odd:
                    forms = _left_forms(ol[M3, c, :, cs], o12[t], x1, x2)
                    for f in (M4, M2, M1, M6, M7):
                        ol[f, c, :, cs] = forms[f]
                else:
                    ol[M3, c, :, cs] = x1
                    ol[M5, c, :, cs] = x1 + x2
                    o12[t] = x2

        project(0, 0)
        project(1, 0)
        for g in range(1, NG):
            project(0, g)
            scores(g - 1)
            project(1, g)
            if g > 1:
                values(g - 2)
            project(2, g - 1)
        project(2, NG - 1)
        order = [(c, n, q) for n in range(2) for c in (0, 1) for q in out_plan[odd]]
        order += [(c, n, q) for c in (2, 3) for n in range(2) for q in out_plan[odd]]
        for i, (c, n, q) in enumerate(order):
            if i == 1:
                scores(NG - 1)
            if i == 5:
                values(NG - 2)
            if i == 15:
                values(NG - 1)
            y = out_product(*q, c, n)
            acc[n, q[0]] = acc[n, q[0]] + y if c else y
        res = []
        for n in range(2):
            out_tokens(n, {f: acc[n, f][n_mem:] for f, _, _ in out_plan[odd]})
            res.append(mem_result({f: acc[n, f][:n_mem] for f, _, _ in out_plan[odd]}))
        return jnp.concatenate([res[0][0], res[1][0], res[0][1], res[1][1]], axis=1), top

    n_blk = n_seg // _BLK

    def out_copy(b):
        r = _rows(b * _BLK * seg, _BLK * seg)
        return pltpu.make_async_copy(ob.at[r], out_hbm.at[r], out_sem)

    def steps(b, carry):
        job = jnp.where(b + 1 < n_blk, b + 1, 0) * (_BLK // 2)
        n_kept = 3 * H // 2 - kept
        for u in range(_BLK):
            carry = step(b, u, carry)
            if u + 1 < _BLK:
                for j in range(n_kept * u // (_BLK - 1), n_kept * (u + 1) // (_BLK - 1)):
                    ahead(kept + j, 1, job, _BLK // 2)

        @pl.when(b == 0)
        def _():
            third.wait()

        @pl.when(b > 0)
        def _():
            out_copy(b - 1).start()

        @pl.when(b == 1)
        def _():
            for cp in ffn:
                cp.start()
        return carry

    ninf = jnp.full((8, 128), -jnp.inf, F32)
    _, top = lax.fori_loop(0, n_blk, steps, (mem_ref[...].astype(F32), (ninf, sub, ninf, sub + 8)))

    for cp in ffn:
        cp.wait()
    for n in range(2):
        out_tokens(n, {q[0]: sum(out_product(*q, c, n, False) for c in range(4)) for q in out_plan[0]})
    for i in range(4):
        top = finish(n_seg - 2, i, None, top)
    out_copy(n_blk - 1).start()

    b1, i1, b2, i2 = top
    t1 = jnp.min(jnp.where(b1 == jnp.max(b1, axis=0, keepdims=True), i1, S), axis=0, keepdims=True)
    b1, i1 = jnp.where(i1 == t1, b2, b1), jnp.where(i1 == t1, i2, i1)
    t2 = jnp.min(jnp.where(b1 == jnp.max(b1, axis=0, keepdims=True), i1, S), axis=0, keepdims=True)
    idx = [jnp.clip(t[0, 0], 0, S - 1) for t in (t1, t2)]
    base = [pl.multiple_of(i // 16 * 16, 16) for i in idx]
    h, hn = (jnp.concatenate([hs[k, pl.ds(r, 16), :] for r in base], axis=0) for k in range(2))
    gate = _rb(jnp.dot(hn.astype(BF16), wg[...], preferred_element_type=F32))
    up = _rb(jnp.dot(hn.astype(BF16), wu[...], preferred_element_type=F32))
    act = _rb(gate * _rb(jax.nn.sigmoid(gate))) * up
    y = _rb(jnp.dot(act.astype(BF16), wd[...], preferred_element_type=F32))
    y = _rb(y * _rb(jax.nn.sigmoid(_rb(jnp.sum(hn * wr, axis=-1, keepdims=True)))))
    ri = lax.broadcasted_iota(jnp.int32, (32, D), 0)
    ri = jnp.where(ri < 16, ri + base[0], ri + (base[1] - 16))
    fix[...] = (h + _rb(hn + jnp.where((ri == idx[0]) | (ri == idx[1]), y, 0.0))).astype(BF16)
    pltpu.make_async_copy(ob, out_hbm, out_sem).wait()
    patch = [pltpu.make_async_copy(fix.at[pl.ds(16 * i, 16)], out_hbm.at[pl.ds(base[i], 16)], sem.at[9 + i])
             for i in range(2)]
    patch[0].start()

    @pl.when(base[0] != base[1])
    def _():
        patch[1].start()
        patch[1].wait()
    patch[0].wait()


@functools.partial(jax.jit, static_argnames=("A_seg_len",))
def pallas_sequential_preLN__memory_aug_recurrent_mem_tr__moe_arch_mod__prompt_kernel(
    A_x, A_mem0, A_Wq, A_Wk, A_Wv, A_Wo, A_seg_len, B_x, B_w_r, B_w_gate, B_w_up, B_w_down,
):
    del B_x
    B, S, D = A_x.shape
    _, H, Dh = A_Wq.shape
    M = A_mem0.shape[1]
    F = B_w_gate.shape[1]
    seg = int(A_seg_len)
    assert (B, S, D, H, Dh, M, seg) == (1, 2048, 512, 32, 128, 8, 32)
    n_seg = S // seg
    live = seg - _PRE
    any_spec = pl.BlockSpec(memory_space=pl.ANY)
    out = pl.pallas_call(
        _kernel,
        out_shape=jax.ShapeDtypeStruct((S, D), A_x.dtype),
        in_specs=[any_spec] * 10,
        out_specs=any_spec,
        scratch_shapes=[
            pltpu.VMEM((M, D), BF16),
            pltpu.VMEM((D // 128, 128), BF16),
            pltpu.VMEM((n_seg, live, D), BF16),
            pltpu.VMEM((n_seg, _PRE, D), BF16),
            pltpu.VMEM((7, live, D // 2), F32),
            pltpu.VMEM((7, n_seg * _PRE // 4, D // 2), U32),
            pltpu.VMEM((n_seg * _PRE // 2, D // 2), F32),
            pltpu.VMEM((3 * H // _CH, D // 2, 2 * _CH, Dh), BF16),
            pltpu.VMEM((3 * H // 2, 7, D // 4, Dh), U32),
            pltpu.VMEM((3 * H, 2, n_seg * _PRE // 2, Dh), F32),
            pltpu.VMEM((3 * H, live, Dh), F32),
            pltpu.VMEM((3 * H, live, Dh), F32),
            pltpu.VMEM((H, Dh, D), BF16),
            pltpu.VMEM((7, H * Dh // 4, D // 2), U32),
            pltpu.VMEM((7, H // 8, seg, 4 * Dh), F32),
            pltpu.VMEM((3, H // 8, M, 4 * Dh), F32),
            pltpu.VMEM((H // 2, seg, Dh), F32),
            pltpu.VMEM((2 * seg, D), F32),
            pltpu.VMEM((2, S, D), F32),
            pltpu.VMEM((D, F), BF16),
            pltpu.VMEM((D, F), BF16),
            pltpu.VMEM((F, D), BF16),
            pltpu.VMEM((S, D), BF16),
            pltpu.VMEM((32, D), BF16),
            pltpu.VMEM((8, 128), U32),
            pltpu.SemaphoreType.DMA((11 + 3 * H // _CH + H // _G,)),
            pltpu.SemaphoreType.DMA,
        ],
        compiler_params=pltpu.CompilerParams(vmem_limit_bytes=110 * 1024 * 1024),
        name="rmt_mod",
    )(A_x.reshape(n_seg, seg, D), A_mem0.reshape(M, D), A_Wq, A_Wk, A_Wv, A_Wo,
      B_w_r.reshape(D // 128, 128), B_w_gate, B_w_up, B_w_down)
    return out.reshape(1, S, D)
```

```python
import functools

import jax
import jax.numpy as jnp
import numpy as np
from jax import lax
import jax.experimental.pallas as pl
import jax.experimental.pallas.tpu as pltpu

F32 = jnp.float32
BF16 = jnp.bfloat16
U32 = jnp.uint32

_NN = (((1,), (0,)), ((), ()))
_NT = (((1,), (1,)), ((), ()))
_PRE = 8
_BLK = 8
_CH = 8
_G = 4
M1, M2, M3, M4, M5, M6, M7 = range(7)


def _rb(x):
    return x.astype(BF16).astype(F32)


def _layernorm(x):
    n = x.shape[-1]
    m = jnp.sum(x, axis=-1, keepdims=True) * (1.0 / n)
    xc = x - m
    v = jnp.sum(xc * xc, axis=-1, keepdims=True) * (1.0 / n)
    sd = _rb(jnp.sqrt(_rb(_rb(v) + 1e-5)))
    return _rb(_rb(x - _rb(m)) * (1.0 / sd))


def _mm(a, w):
    return lax.dot_general(a, pltpu.bitcast(w, BF16), _NN, preferred_element_type=F32)


def _left_forms(a11, a12, a21, a22):
    return a11 + a22, a21 + a22, a11, a22, a11 + a12, a21 - a11, a12 - a22


def _right_forms(b11, b12, b21, b22):
    f11, f12, f21, f22 = (pltpu.bitcast(b, BF16).astype(F32) for b in (b11, b12, b21, b22))

    def pack(x):
        return pltpu.bitcast(x.astype(BF16), U32)
    return pack(f11 + f22), b11, pack(f12 - f22), pack(f21 - f11), b22, pack(f11 + f12), pack(f21 + f22)


def _swap8(w):
    sub = lax.broadcasted_iota(jnp.int32, w[0].shape, 0)
    u = [pltpu.roll(w[-k % 8], -k % 8, 0) if k else w[0] for k in range(8)]
    for b in (1, 2, 4):
        u = [jnp.where((sub & b) != 0, u[(k - b) % 8], u[k]) for k in range(8)]
    return [pltpu.roll(u[j], -j % 8, 0) if j else u[0] for j in range(8)]


def _rows(start, size):
    return pl.ds(start, size) if isinstance(start, int) else pl.ds(pl.multiple_of(start, size), size)


def _kernel(x_hbm, mem_hbm, wq_hbm, wk_hbm, wv_hbm, wo_hbm, wr_hbm, wg_hbm, wu_hbm, wd_hbm,
            out_hbm,
            mem_ref, wr_ref, xa, xb, xl, xp, xg, raw, wp, pre, part, nxt, wo_raw, wo, ol, om, o12, att, fin, hs,
            wg, wu, wd, ob, fix, zero, sem, out_sem):
    n_seg, seg, D = x_hbm.shape
    _, H, dh = wq_hbm.shape
    S = n_seg * seg
    n_job = n_seg // 2
    n_mem = mem_ref.shape[0]
    live = seg - _PRE
    half = D // 2
    NG = H // _G
    NC = 3 * H // _CH

    def w_start(c, d0, n, s):
        w = (wk_hbm, wq_hbm, wv_hbm)[c * _CH // H]
        for i in range(2):
            pltpu.make_async_copy(w.at[pl.ds(i * half + d0, n), pl.ds(c * _CH % H, _CH), :],
                                  raw.at[c, pl.ds(d0, n), pl.ds(i * _CH, _CH), :], sem.at[s]).start()

    def w_wait(c, d0, n, s):
        pltpu.make_async_copy(raw.at[c, pl.ds(d0, n)], raw.at[c, pl.ds(d0, n)], sem.at[s]).wait()

    def chunk(c):
        return c, 0, half, 11 + c

    def last_chunk(g):
        return NC - 1, g * (half // NG), half // NG, 10 + NC + g

    def wo_copy(g):
        r = pl.ds(g * _G, _G)
        return pltpu.make_async_copy(wo_hbm.at[r], wo_raw.at[r], sem.at[10 + NC + NG + g])

    def xa_copy(i, lo, hi):
        r = pl.ds(lo, hi - lo)
        return pltpu.make_async_copy(x_hbm.at[r, pl.ds(0, live), :], xa.at[r], sem.at[i])

    first = [pltpu.make_async_copy(x_hbm.at[:, pl.ds(live, _PRE), :], xb, sem.at[0]), xa_copy(1, 0, 2)]
    second = [pltpu.make_async_copy(mem_hbm, mem_ref, sem.at[2]), pltpu.make_async_copy(wr_hbm, wr_ref, sem.at[3]),
              xa_copy(4, 2, 2 * _BLK)]
    third = xa_copy(5, 2 * _BLK, n_seg)
    ffn = [pltpu.make_async_copy(a, b, sem.at[6 + i])
           for i, (a, b) in enumerate(((wg_hbm, wg), (wu_hbm, wu), (wd_hbm, wd)))]
    wo_from = NC - 1 - NG
    for cp in first:
        cp.start()
    for c in range(NC - 1):
        w_start(*chunk(c))
        if c >= wo_from:
            w_start(*last_chunk(c - wo_from))
            wo_copy(c - wo_from).start()
    for cp in second + [third]:
        cp.start()

    def pace(y):
        return pltpu.bitcast(y, U32) & zero[...]

    def prepare_qkv(c, i, after):
        a = pltpu.bitcast(raw[c, pl.ds(i * 16, 16)], U32).reshape(8, 2, _CH, dh)
        t = []
        for b in range(2):
            e, o = (a[:, k] if after is None else a[:, k] | after[b] for k in range(2))
            w = (e >> 16) | (o & np.uint32(0xFFFF0000)) if b else (e & np.uint32(0xFFFF)) | (o << 16)
            t.append(_swap8([w[j] for j in range(8)]))
        n = _CH // 2
        for j in range(n):
            blocks = [t[0][j], t[1][j], t[0][n + j], t[1][n + j]]
            if after is not None:
                blocks = [x | after[2 + j // 2] for x in blocks]
            for f, w in enumerate(_right_forms(*blocks)):
                wp[c * n + j, f, _rows(i * 8, 8), :] = w

    def prepare_wo(g, i, after):
        pair, j = i // 8, i % 8
        top, bot = (pltpu.bitcast(wo_raw[g * _G + 2 * pair + b, pl.ds(j * 16, 16), :], U32)
                    | jnp.tile(after, (1, D // 128)) for b in range(2))
        forms = _right_forms(top[:, :half], top[:, half:], bot[:, :half], bot[:, half:])
        for f, w in enumerate(forms):
            wo[f, _rows(g * dh + i * 8, 8), :] = w

    def live_forms(job, j):
        r = pl.ds(j * 8, 8)
        top, bot = (_layernorm(xa[2 * job + b, r].astype(F32)) for b in range(2))
        forms = _left_forms(top[:, :half], top[:, half:], bot[:, :half], bot[:, half:])
        for f, v in enumerate(forms):
            if f == M2 and j == 2:
                xg[0, _rows(job * 8, 8), :] = v
            else:
                xl[f, r, :] = v
        return forms[M1][:, :128]

    def ahead(pair, n_pair, job, n, start=False):
        r = n * _PRE

        def product(j, f):
            lhs = pltpu.bitcast(xp[f, _rows(job * (_PRE // 2), r // 2), :], BF16)
            if start and f in (M1, M6, M7):
                lhs = jnp.concatenate([lhs, xl[f].astype(BF16)], axis=0)
            return _mm(lhs, wp[pair + j, f])
        if n_pair == 1:
            order = [(0, f) for f in (M1, M6, M7, M4, M3, M5)]
        else:
            order = [(0, M1), (0, M6), (0, M7), (1, M7), (0, M4), (1, M4), (0, M3), (0, M5),
                     (1, M1), (1, M6), (1, M3), (1, M5)]
        m = {jf: product(*jf) for jf in order}
        rows = _rows(job * _PRE, r)
        for j in range(n_pair):
            t = 2 * (pair + j)
            c11, c22 = m[j, M1] + m[j, M7], m[j, M1] + m[j, M6]
            if start:
                part[t] = c11[r:]
                part[t + 1] = c22[r:]
            pre[t, 0, rows, :] = c11[:r] + m[j, M4] - m[j, M5]
            pre[t + 1, 0, rows, :] = m[j, M3] + m[j, M5]
            pre[t, 1, rows, :] = m[j, M4]
            pre[t + 1, 1, rows, :] = c22[:r] + m[j, M3]
        return [m[jf] for jf in order[::2]]

    zero[...] = jnp.zeros(zero.shape, U32)
    att[...] = jnp.zeros(att.shape, F32)
    fin[...] = jnp.zeros(fin.shape, F32)
    for f in (M1, M2, M6, M7):
        ol[f] = jnp.zeros(ol.shape[1:], F32)
    for cp in first:
        cp.wait()

    def pre_forms(i, _):
        n = n_job // 2
        v = _layernorm(xb[pl.ds(i * 2 * n, 2 * n)].astype(F32).reshape(2 * n * _PRE, D)).reshape(n, 2, _PRE, D)
        top, bot = (v[:, b].reshape(n * _PRE, D) for b in range(2))
        for f, u in enumerate(_left_forms(top[:, :half], top[:, half:], bot[:, :half], bot[:, half:])):
            if f == M2:
                xg[1, _rows(i * n * _PRE, n * _PRE), :] = u
            else:
                xp[f, _rows(i * n * _PRE // 2, n * _PRE // 2), :] = pltpu.bitcast(u.astype(BF16), U32)
    lax.fori_loop(0, 2, pre_forms, None)
    for j in range(live // 8):
        live_forms(0, j)

    w_wait(*chunk(0))
    lax.fori_loop(0, half // 16, lambda i, _: prepare_qkv(0, i, None), None)

    def prologue(with_rest, c, _):
        w_wait(*chunk(c))
        if with_rest:
            w_wait(*last_chunk(c - wo_from))
            wo_copy(c - wo_from).wait()
        z = [pace(y[r:r + 8]) for j in (0, 2) for y in ahead(c * (_CH // 2) + (j - _CH // 2), 2, 0, n_job, True)
             for r in range(0, 256, 32)]
        for i in range(half // 16):
            prepare_qkv(c, i, z[5 * i:5 * i + 4])
            if with_rest:
                prepare_wo(c - wo_from, i, z[5 * i + 4])
        if with_rest:
            for i in range(2):
                prepare_qkv(NC - 1, (c - wo_from) * 2 + i, z[80 + 5 * i:84 + 5 * i])
    lax.fori_loop(1, wo_from, functools.partial(prologue, False), None)
    lax.fori_loop(wo_from, NC - 1, functools.partial(prologue, True), None)

    kept = (NC - 2) * (_CH // 2)
    for cp in second:
        cp.wait()
    for pair in range(kept, 3 * H // 2, 2):
        ahead(pair, 2, 0, _BLK // 2, True)

    def pos(i):
        return jnp.where(i < live, i + n_mem, jnp.where(i < live + n_mem, i - live, i))
    row = pos(lax.broadcasted_iota(jnp.int32, (seg + n_mem, seg + n_mem), 0))
    col = pos(lax.broadcasted_iota(jnp.int32, (seg + n_mem, seg + n_mem), 1))
    mask = (row < n_mem) | (row >= col)
    scale = float(dh) ** -0.5

    wr = wr_ref[...].astype(F32)
    wr = jnp.concatenate([wr[i:i + 1, :] for i in range(D // 128)], axis=1)
    sub = lax.broadcasted_iota(jnp.int32, (8, 128), 0)

    def finish(s0, i, valid, top):
        b1, i1, b2, i2 = top
        s = s0 + i // 2
        if i % 2 == 0:
            x = xa[s, 0:16].astype(F32)
        else:
            x = jnp.concatenate([xa[s, 16:live].astype(F32), xb[s].astype(F32)], axis=0)
        r = _rows(s0 * seg + i * 16, 16)
        h = _rb(x + _rb(fin[i * 16:i * 16 + 16]))
        hn = _layernorm(h)
        hs[0, r, :] = h
        hs[1, r, :] = hn
        ob[r, :] = (h + hn).astype(BF16)
        score = _rb(jnp.sum(hn * wr, axis=-1, keepdims=True))
        for j in range(2):
            val = jnp.broadcast_to(score[8 * j:8 * j + 8], (8, 128))
            if valid is not None:
                val = jnp.where(valid, val, -jnp.inf)
            idx = sub + (s0 * seg + i * 16 + 8 * j)
            g1 = val > b1
            g2 = val > b2
            b2 = jnp.where(g1, b1, jnp.where(g2, val, b2))
            i2 = jnp.where(g1, i1, jnp.where(g2, idx, i2))
            b1 = jnp.where(g1, val, b1)
            i1 = jnp.where(g1, idx, i1)
        return b1, i1, b2, i2

    mem_operand = {M1: 1, M2: 2, M3: 0, M4: 1, M5: 2, M6: 0, M7: 1}

    def mem_result(m):
        if M3 in m:
            return m[M2] + m[M4], m[M3] + m[M5]
        d = m[M2] - m[M1]
        return m[M7] + d, m[M6] - d

    hseg = seg // 2
    out_plan = (((M1, 0, seg), (M6, 0, seg), (M2, hseg, seg), (M7, 0, seg)),
                ((M4, 0, seg), (M3, 0, seg), (M2, 0, hseg), (M5, 0, seg)))

    def out_product(f, r0, r1, c, n, with_mem=True):
        lhs = ol[f, c, r0:r1]
        if with_mem:
            lhs = jnp.concatenate([om[mem_operand[f], c], lhs], axis=0)
        return _mm(lhs, wo[f, c * 2 * dh:(c + 1) * 2 * dh, n * 128:(n + 1) * 128])

    def out_tokens(n, m):
        lo, hi = pl.ds(n * 128, 128), pl.ds(half + n * 128, 128)
        if M3 in m:
            att[0:seg, lo] = m[M4] - m[M5]
            att[0:seg, hi] = m[M3] + m[M5]
            att[seg:seg + hseg, lo] = m[M4][:hseg] + m[M2]
            att[seg + hseg:2 * seg, lo] = m[M4][hseg:]
            att[seg:seg + hseg, hi] = m[M3][:hseg] - m[M2]
            att[seg + hseg:2 * seg, hi] = m[M3][hseg:]
        else:
            fin[0:seg, lo] = att[0:seg, lo] + (m[M1] + m[M7])
            fin[0:seg, hi] = att[0:seg, hi]
            fin[seg:seg + hseg, lo] = att[seg:seg + hseg, lo]
            fin[seg + hseg:2 * seg, lo] = att[seg + hseg:2 * seg, lo] + m[M2]
            t = m[M1] + m[M6]
            fin[seg:seg + hseg, hi] = att[seg:seg + hseg, hi] + t[:hseg]
            fin[seg + hseg:2 * seg, hi] = att[seg + hseg:2 * seg, hi] + (t[hseg:] - m[M2])

    def step(b, u, carry):
        mem, top = carry
        odd = u % 2
        job = b * (_BLK // 2) + u // 2
        pr = _rows(job * _PRE, _PRE)
        a = (mem[:, :half], mem[:, half:], mem[:, :half] + mem[:, half:])
        lhs = {f: jnp.concatenate([xl[f], a[mem_operand[f]]], axis=0).astype(BF16)
               for f in ((M1, M6, M7) if odd else (M4, M3, M5))}
        order = [(j, f) for j in range(2) for f in lhs]
        lhs[M2] = jnp.concatenate(([xg[0, pr, :], xg[1, pr, :]] if odd else [xl[M2, 0:16]]) + [a[2]], axis=0)
        needs = {}
        if not odd:
            s0, valid = (jnp.maximum(2 * job - 4, 0), b > 0) if u < 4 else (2 * job - 4, None)
            for i in range(4):
                top = finish(s0, i, valid, top)
                needs[1, 1 + i] = top[3]
            nj = jnp.where(job + 1 < n_job, job + 1, 0) if u + 2 == _BLK else job + 1
            for i in range(live // 8):
                needs[1, 5 + i] = live_forms(nj, i)
        kqv, p, acc = ({}, {}, {}), {}, {}

        def project(w, g):
            t0 = w * H + g * _G
            early = [pre[t, odd, pr, :] for t in range(t0, t0 + _G)]
            if (w, g) in needs:
                early[0] = pltpu.bitcast(pltpu.bitcast(early[0], U32) | pace(needs[w, g]), F32)
            at = 6 if w else 2
            y = {(j, f): _mm(lhs[f], wp[t0 // 2 + j, f]) for j, f in order[:at] + [(0, M2), (1, M2)] + order[at:]}
            for j in range(2):
                t = t0 + 2 * j
                m = {f: y[j, f][:-n_mem] for f in lhs}
                c1, c2 = mem_result({f: y[j, f][-n_mem:] for f in lhs})
                if odd:
                    rows = ((nxt[t, 0:16], nxt[t, 16:live] + m[M2][:8], c1, early[2 * j] + m[M2][8:]),
                            (nxt[t + 1, 0:16], nxt[t + 1, 16:live] - m[M2][:8], c2, early[2 * j + 1] - m[M2][8:]))
                    part[t] = m[M1] + m[M7]
                    part[t + 1] = m[M1] + m[M6]
                else:
                    rows = ((part[t] + (m[M4] - m[M5]), c1, early[2 * j]), (m[M3] + m[M5], c2, early[2 * j + 1]))
                    c22 = part[t + 1] + m[M3]
                    nxt[t] = jnp.concatenate([m[M4][:16] + m[M2], m[M4][16:]], axis=0)
                    nxt[t + 1] = jnp.concatenate([c22[:16] - m[M2], c22[16:]], axis=0)
                for i in range(2):
                    kqv[w][g * _G + 2 * j + i] = jnp.concatenate(rows[i], axis=0)

        def scores(g):
            for i in range(g * _G, (g + 1) * _G):
                sc = lax.dot_general(kqv[1][i], kqv[0][i].astype(BF16), _NT, preferred_element_type=F32)
                sc = jnp.where(mask, sc, -1e9 / scale)
                e = jnp.exp2((sc - jnp.max(sc, axis=-1, keepdims=True)) * (scale * float(np.log2(np.e))))
                l = jnp.sum(e, axis=-1, keepdims=True)
                r = pl.reciprocal(l, approx=True)
                p[i] = e * (r * (2.0 - l * r))

        def values(g):
            o = [lax.dot_general(p[i], kqv[2][i].astype(BF16), _NN, preferred_element_type=F32)
                 for i in range(g * _G, (g + 1) * _G)]
            for j in range(2):
                t = 2 * g + j
                c, cs = t // 4, pl.ds((t % 4) * dh, dh)
                m1, m2 = (x[live:live + n_mem] for x in o[2 * j:2 * j + 2])
                om[0, c, :, cs] = m1
                om[1, c, :, cs] = m2
                om[2, c, :, cs] = m1 + m2
                x1, x2 = (jnp.concatenate([x[:live], x[live + n_mem:]], axis=0) for x in o[2 * j:2 * j + 2])
                if odd:
                    forms = _left_forms(ol[M3, c, :, cs], o12[t], x1, x2)
                    for f in (M4, M2, M1, M6, M7):
                        ol[f, c, :, cs] = forms[f]
                else:
                    ol[M3, c, :, cs] = x1
                    ol[M5, c, :, cs] = x1 + x2
                    o12[t] = x2

        for g in range(NG):
            project(0, g)
            project(1, g)
            if g > 1:
                values(g - 2)
            project(2, g)
            scores(g)
        units = [(c, n, q) for n in range(2) for c in (0, 1) for q in out_plan[odd]]
        units += [(c, n, q) for c in (2, 3) for n in range(2) for q in out_plan[odd]]
        for i, (c, n, q) in enumerate(units):
            if i == 4:
                values(NG - 2)
            if i == 15:
                values(NG - 1)
            y = out_product(*q, c, n)
            acc[n, q[0]] = acc[n, q[0]] + y if c else y
        res = []
        for n in range(2):
            out_tokens(n, {f: acc[n, f][n_mem:] for f, _, _ in out_plan[odd]})
            res.append(mem_result({f: acc[n, f][:n_mem] for f, _, _ in out_plan[odd]}))
        return jnp.concatenate([res[0][0], res[1][0], res[0][1], res[1][1]], axis=1), top

    n_blk = n_seg // _BLK

    def out_copy(b):
        r = _rows(b * _BLK * seg, _BLK * seg)
        return pltpu.make_async_copy(ob.at[r], out_hbm.at[r], out_sem)

    def steps(b, carry):
        job = jnp.where(b + 1 < n_blk, b + 1, 0) * (_BLK // 2)
        n_kept = 3 * H // 2 - kept
        for u in range(_BLK):
            carry = step(b, u, carry)
            if u + 1 < _BLK:
                for j in range(n_kept * u // (_BLK - 1), n_kept * (u + 1) // (_BLK - 1)):
                    ahead(kept + j, 1, job, _BLK // 2)

        @pl.when(b == 0)
        def _():
            third.wait()

        @pl.when(b > 0)
        def _():
            out_copy(b - 1).start()

        @pl.when(b == 1)
        def _():
            for cp in ffn:
                cp.start()
        return carry

    ninf = jnp.full((8, 128), -jnp.inf, F32)
    _, top = lax.fori_loop(0, n_blk, steps, (mem_ref[...].astype(F32), (ninf, sub, ninf, sub + 8)))

    for cp in ffn:
        cp.wait()
    for i in range(4):
        top = finish(n_seg - 4, i, None, top)
    for n in range(2):
        out_tokens(n, {q[0]: sum(out_product(*q, c, n, False) for c in range(4)) for q in out_plan[0]})
    for i in range(4):
        top = finish(n_seg - 2, i, None, top)
    out_copy(n_blk - 1).start()

    b1, i1, b2, i2 = top
    t1 = jnp.min(jnp.where(b1 == jnp.max(b1, axis=0, keepdims=True), i1, S), axis=0, keepdims=True)
    b1, i1 = jnp.where(i1 == t1, b2, b1), jnp.where(i1 == t1, i2, i1)
    t2 = jnp.min(jnp.where(b1 == jnp.max(b1, axis=0, keepdims=True), i1, S), axis=0, keepdims=True)
    idx = [jnp.clip(t[0, 0], 0, S - 1) for t in (t1, t2)]
    base = [pl.multiple_of(i // 16 * 16, 16) for i in idx]
    h, hn = (jnp.concatenate([hs[k, pl.ds(r, 16), :] for r in base], axis=0) for k in range(2))
    gate = _rb(jnp.dot(hn.astype(BF16), wg[...], preferred_element_type=F32))
    up = _rb(jnp.dot(hn.astype(BF16), wu[...], preferred_element_type=F32))
    act = _rb(gate * _rb(jax.nn.sigmoid(gate))) * up
    y = _rb(jnp.dot(act.astype(BF16), wd[...], preferred_element_type=F32))
    y = _rb(y * _rb(jax.nn.sigmoid(_rb(jnp.sum(hn * wr, axis=-1, keepdims=True)))))
    ri = lax.broadcasted_iota(jnp.int32, (32, D), 0)
    ri = jnp.where(ri < 16, ri + base[0], ri + (base[1] - 16))
    fix[...] = (h + _rb(hn + jnp.where((ri == idx[0]) | (ri == idx[1]), y, 0.0))).astype(BF16)
    pltpu.make_async_copy(ob, out_hbm, out_sem).wait()
    patch = [pltpu.make_async_copy(fix.at[pl.ds(16 * i, 16)], out_hbm.at[pl.ds(base[i], 16)], sem.at[9 + i])
             for i in range(2)]
    patch[0].start()

    @pl.when(base[0] != base[1])
    def _():
        patch[1].start()
        patch[1].wait()
    patch[0].wait()


@functools.partial(jax.jit, static_argnames=("A_seg_len",))
def pallas_sequential_preLN__memory_aug_recurrent_mem_tr__moe_arch_mod__prompt_kernel(
    A_x, A_mem0, A_Wq, A_Wk, A_Wv, A_Wo, A_seg_len, B_x, B_w_r, B_w_gate, B_w_up, B_w_down,
):
    del B_x
    B, S, D = A_x.shape
    _, H, Dh = A_Wq.shape
    M = A_mem0.shape[1]
    F = B_w_gate.shape[1]
    seg = int(A_seg_len)
    assert (B, S, D, H, Dh, M, seg) == (1, 2048, 512, 32, 128, 8, 32)
    n_seg = S // seg
    live = seg - _PRE
    any_spec = pl.BlockSpec(memory_space=pl.ANY)
    out = pl.pallas_call(
        _kernel,
        out_shape=jax.ShapeDtypeStruct((S, D), A_x.dtype),
        in_specs=[any_spec] * 10,
        out_specs=any_spec,
        scratch_shapes=[
            pltpu.VMEM((M, D), BF16),
            pltpu.VMEM((D // 128, 128), BF16),
            pltpu.VMEM((n_seg, live, D), BF16),
            pltpu.VMEM((n_seg, _PRE, D), BF16),
            pltpu.VMEM((7, live, D // 2), F32),
            pltpu.VMEM((7, n_seg * _PRE // 4, D // 2), U32),
            pltpu.VMEM((2, n_seg * _PRE // 2, D // 2), F32),
            pltpu.VMEM((3 * H // _CH, D // 2, 2 * _CH, Dh), BF16),
            pltpu.VMEM((3 * H // 2, 7, D // 4, Dh), U32),
            pltpu.VMEM((3 * H, 2, n_seg * _PRE // 2, Dh), F32),
            pltpu.VMEM((3 * H, live, Dh), F32),
            pltpu.VMEM((3 * H, live, Dh), F32),
            pltpu.VMEM((H, Dh, D), BF16),
            pltpu.VMEM((7, H * Dh // 4, D // 2), U32),
            pltpu.VMEM((7, H // 8, seg, 4 * Dh), F32),
            pltpu.VMEM((3, H // 8, M, 4 * Dh), F32),
            pltpu.VMEM((H // 2, seg, Dh), F32),
            pltpu.VMEM((2 * seg, D), F32),
            pltpu.VMEM((2 * seg, D), F32),
            pltpu.VMEM((2, S, D), F32),
            pltpu.VMEM((D, F), BF16),
            pltpu.VMEM((D, F), BF16),
            pltpu.VMEM((F, D), BF16),
            pltpu.VMEM((S, D), BF16),
            pltpu.VMEM((32, D), BF16),
            pltpu.VMEM((8, 128), U32),
            pltpu.SemaphoreType.DMA((10 + 3 * H // _CH + 2 * H // _G,)),
            pltpu.SemaphoreType.DMA,
        ],
        compiler_params=pltpu.CompilerParams(vmem_limit_bytes=110 * 1024 * 1024),
        name="rmt_mod",
    )(A_x.reshape(n_seg, seg, D), A_mem0.reshape(M, D), A_Wq, A_Wk, A_Wv, A_Wo,
      B_w_r.reshape(D // 128, 128), B_w_gate, B_w_up, B_w_down)
    return out.reshape(1, S, D)
```
